```python
import os as _os
_os.environ.setdefault("JAX_PLATFORMS", "cpu")
import jax
import jax.numpy as jnp

def _softmax(x, axis=-1):
    return jax.nn.softmax(x, axis=axis)
def _gelu(x):
    return jax.nn.gelu(x, approximate=True)
def _silu(x):
    return jax.nn.silu(x)
def _sigmoid(x):
    return jax.nn.sigmoid(x)
def _layernorm(x, axis=-1, eps=1e-5):
    m = jnp.mean(x, axis=axis, keepdims=True)
    v = jnp.var(x, axis=axis, keepdims=True)
    return (x - m) / jnp.sqrt(v + eps)
def _scatter_add(tgt, idx, src, axis=0):
    return tgt.at[idx].add(src)
def _segment_sum(src, seg, n):
    return jax.ops.segment_sum(src, seg, n)
class _Rng:
    def __init__(self, key):
        self._k = key
    def _next(self):
        self._k, sub = jax.random.split(self._k)
        return sub
    def normal(self, shape):
        return jax.random.normal(self._next(), shape, dtype=jnp.bfloat16)
    def randint(self, lo, hi, shape):
        return jax.random.randint(self._next(), shape, lo, hi, dtype=jnp.int32)
    def uniform(self, shape, lo=0.0, hi=1.0):
        return jax.random.uniform(self._next(), shape, jnp.bfloat16, lo, hi)
    def permutation(self, n):
        return jax.random.permutation(self._next(), n)


kernel_name = 'sequential_preLN__softmax_full_mha__glu_gated_swiglu__prompt'

def setup_inputs():
    _rng = _Rng(jax.random.key(int.from_bytes(__import__("os").urandom(4), "little")))
    _w = (lambda a: (lambda t: t.astype(jnp.bfloat16) if jnp.issubdtype(t.dtype, jnp.floating) else t)(jnp.asarray(a)))
    def _A_setup():
        B, S, D = 1, 2048, 512
        return {
            "x": _w((lambda *s: _rng.normal(s) * 0.05)(B, S, D)),
            "wqkv": _w((lambda *s: _rng.normal(s) * 0.05)(D, 3 * D)),
            "wo": _w((lambda *s: _rng.normal(s) * 0.05)(D, D)),
        }
    _A_in = _A_setup()

    def _B_setup():
        B, S, D, F = 1, 2048, 512, 1376
        return {
            "x": _w((lambda *s: _rng.normal(s) * 0.05)(B, S, D)),
            "w1": _w((lambda *s: _rng.normal(s) * 0.05)(D, F) * (2.0 / D) ** 0.5),
            "w3": _w((lambda *s: _rng.normal(s) * 0.05)(D, F) * (2.0 / D) ** 0.5),
            "w2": _w((lambda *s: _rng.normal(s) * 0.05)(F, D) * (2.0 / F) ** 0.5),
        }
    _B_in = _B_setup()

    return {
        "A_x": _A_in["x"],
        "A_wqkv": _A_in["wqkv"],
        "A_wo": _A_in["wo"],
        "B_x": _B_in["x"],
        "B_w1": _B_in["w1"],
        "B_w3": _B_in["w3"],
        "B_w2": _B_in["w2"],
    }

def reference(A_x, A_wqkv, A_wo, B_x, B_w1, B_w3, B_w2):
    def _A_ref(x, wqkv, wo):
        B, S, D = x.shape
        H = 32; Dh = D // H
        qkv = (lambda x, *d: x.transpose(*d))((x @ wqkv).reshape(B, S, 3, H, Dh), 2, 0, 3, 1, 4)
        q, k, v = qkv[0], qkv[1], qkv[2]
        scale = Dh ** -0.5
        scores = jnp.einsum("bhqd,bhkd->bhqk", q, k) * scale
        p = _softmax(scores, axis=-1)
        o = jnp.einsum("bhqk,bhkd->bhqd", p, v)
        return (lambda x, *d: x.transpose(*d))(o, 0, 2, 1, 3).reshape(B, S, D) @ wo

    def _B_ref(x, w1, w3, w2):
        gate = jnp.einsum("bsd,df->bsf", x, w1)
        up = jnp.einsum("bsd,df->bsf", x, w3)
        h = _silu(gate) * up
        out = jnp.einsum("bsf,fd->bsd", h, w2)
        return out

    x = A_x
    h = x + _A_ref(_layernorm(x, axis=-1), A_wqkv, A_wo)
    h2 = h + _B_ref(_layernorm(h, axis=-1), B_w1, B_w3, B_w2)
    return h2
```

```python
import math

import jax
import jax.numpy as jnp
import jax.experimental.pallas as pl
import jax.experimental.pallas.tpu as pltpu

S = 2048
D = 512
H = 32
DH = 16
F = 1376
TQ = 512
TK = 128
HPB = 8
DEPTH = 2
NQ = S // TQ
NC = S // TK
NG = H // HPB
RC = 512
NR = S // RC
FC = 256
EPS = 1e-5
QSCALE = (DH ** -0.5) * math.log2(math.e)
L_LO = 2.0 ** -64
L_HI = 2.0 ** 64

F32 = jnp.float32
BF16 = jnp.bfloat16


def _tree(op, xs):
    xs = list(xs)
    while len(xs) > 1:
        nxt = [op(xs[i], xs[i + 1]) for i in range(0, len(xs) - 1, 2)]
        if len(xs) % 2:
            nxt.append(xs[-1])
        xs = nxt
    return xs[0]


def _ln(x):
    m = jnp.mean(x, axis=-1, keepdims=True)
    xc = x - m
    v = jnp.mean(xc * xc, axis=-1, keepdims=True)
    return xc * jax.lax.rsqrt(v + EPS)


def _dot(a, b):
    return jnp.dot(a, b, preferred_element_type=F32)


def _dot_nt(a, b):
    return jax.lax.dot_general(a, b, (((1,), (1,)), ((), ())), preferred_element_type=F32)


def _kernel(x_hbm, wqkv_hbm, wo_hbm, w1_hbm, w3_hbm, w2_hbm, out_ref,
            x_v, wq_v, wk_v, wv_v, wo_v, w1_v, w3_v, w2_v,
            ln_s, k_s, vt_s, qt_s, qm_s, ot_s, on_s, m_s, l_s, o_s, lraw_s, sc_s, sems):
    step = pl.program_id(0)

    def x_copy(c):
        return pltpu.make_async_copy(x_hbm.at[0, pl.ds(c * RC, RC), :], x_v.at[pl.ds(c * RC, RC), :], sems.at[c])

    def w_copy(i):
        src, dst = [(wqkv_hbm.at[:, pl.ds(D, D)], wk_v), (wqkv_hbm.at[:, pl.ds(2 * D, D)], wv_v),
                    (wqkv_hbm.at[:, pl.ds(0, D)], wq_v),
                    (wo_hbm, wo_v), (w1_hbm, w1_v), (w3_hbm, w3_v), (w2_hbm, w2_v)][i]
        return pltpu.make_async_copy(src, dst, sems.at[NR + i])

    def sel_matrix():
        head_of = jax.lax.broadcasted_iota(jnp.int32, (H, D), 1) // DH
        return (head_of == jax.lax.broadcasted_iota(jnp.int32, (H, D), 0)).astype(BF16)

    def qk(slot, g, c):
        return _dot(k_s[g, c * TK:(c + 1) * TK, :], qm_s[slot])

    def prep(tile):
        q0 = pl.multiple_of(tile * TQ, TQ)
        qt = qt_s[:, pl.ds(q0, TQ)]
        for h in range(H):
            j = h % 8
            qm_s[h, 16 * j:16 * j + 16, :] = qt[16 * h:16 * h + 16, :]
        q1 = pl.multiple_of(jnp.minimum(tile + 1, NQ - 1) * TQ, TQ)
        qm_s[H, 0:16, :] = qt_s[0:16, pl.ds(q1, TQ)]

    @pl.when(step == 0)
    def _prologue():
        x_copy(0).start()
        w_copy(0).start()
        for c in range(1, NR):
            x_copy(c).start()
        w_copy(1).start()
        w_copy(2).start()
        qm_s[...] = jnp.zeros(qm_s.shape, qm_s.dtype)
        ot_s[...] = jnp.zeros(ot_s.shape, ot_s.dtype)
        o_s[...] = jnp.zeros(o_s.shape, F32)
        lraw_s[...] = jnp.ones(lraw_s.shape, F32)

        def ln_chunk(c):
            rows = slice(c * RC, (c + 1) * RC)
            ln_s[rows, :] = _ln(x_v[rows, :].astype(F32)).astype(BF16)

        def k_chunk(c):
            rows = slice(c * RC, (c + 1) * RC)
            k = _dot(ln_s[rows, :], wk_v[...]).astype(BF16)
            for g in range(4):
                k_s[g, rows, :] = k[:, 128 * g:128 * (g + 1)]
            kf = k.astype(F32)
            return (kf * kf).astype(BF16)

        x_copy(0).wait()
        ln_chunk(0)
        w_copy(0).wait()
        x_copy(1).wait()
        ksq = [k_chunk(0)]
        ln_chunk(1)
        x_copy(2).wait()
        ksq.append(k_chunk(1))
        ln_chunk(2)
        x_copy(3).wait()
        w_copy(1).wait()
        w_copy(2).wait()
        for i in range(3, 7):
            w_copy(i).start()
        ksq.append(k_chunk(2))
        ln_chunk(3)
        wvt = wv_v[...].T
        wqt = wq_v[...].T
        ksq.append(k_chunk(3))
        kmax = None
        for c in range(NR):
            kn2 = _dot_nt(sel_matrix(), ksq[c])
            kmax = kn2 if kmax is None else jnp.maximum(kmax, kn2)
        kmax = jnp.max(kmax, axis=1, keepdims=True)
        qsq = []
        for c in range(NR):
            rows = slice(c * RC, (c + 1) * RC)
            q = (_dot_nt(wqt, ln_s[rows, :]) * QSCALE).astype(BF16)
            qt_s[:, rows] = q
            qf = q.astype(F32)
            qsq.append((qf * qf).astype(BF16))
        prep(0)
        for t in range(DEPTH):
            sc_s[t] = qk(0, 0, t)
        for c in range(NR):
            rows = slice(c * RC, (c + 1) * RC)
            vt_s[:, rows] = _dot_nt(wvt, ln_s[rows, :]).astype(BF16)
            qn2 = _dot(sel_matrix(), qsq[c])
            m_s[:, rows] = jnp.sqrt(qn2 * kmax) * 1.02
        for i in range(3, 7):
            w_copy(i).wait()

    q0 = pl.multiple_of(step * TQ, TQ)

    def pv(h, c, s, m, l_acc, o_acc):
        p = jnp.exp2(s - m)
        ll = _tree(jnp.add, [p[8 * i:8 * i + 8] for i in range(TK // 8)])
        l_acc = ll if l_acc is None else l_acc + ll
        vt = vt_s[pl.ds(pl.multiple_of(h * DH, DH), DH), c * TK:(c + 1) * TK]
        oo = _dot(vt, p.astype(BF16))
        o_acc = oo if o_acc is None else o_acc + oo
        return l_acc, o_acc

    def finalize(h, l_acc, o_acc):
        l = l_acc.sum(0, keepdims=True)
        l_s[pl.ds(h, 1), :] = l
        ot_s[pl.ds(pl.multiple_of(h * DH, DH), DH), :] = (o_acc * pl.reciprocal(l, approx=False)).astype(BF16)

    def untranspose(g):
        on_s[g] = ot_s[pl.ds(pl.multiple_of(g * 128, 128), 128), :].T

    def fast_body(i, carry):
        finalize(jnp.maximum(i * HPB - 1, 0), lraw_s[...], o_s[...])
        untranspose(jnp.maximum(i - 1, 0))
        items = [(i * HPB + j, i, c) for j in range(HPB) for c in range(NC)]
        last = i == NG - 1
        nslot = jnp.where(last, H, (i + 1) * HPB)
        ng = jnp.where(last, 0, i + 1)
        items_all = items + [(nslot, ng, c) for c in range(DEPTH)]
        ss = {t: sc_s[t] for t in range(DEPTH)}
        m = l_acc = o_acc = None
        for t, (h, g, c) in enumerate(items):
            ss[t + DEPTH] = qk(*items_all[t + DEPTH])
            if c == 0:
                m = m_s[pl.ds(h, 1), pl.ds(q0, TQ)]
                l_acc = o_acc = None
            l_acc, o_acc = pv(h, c, ss.pop(t), m, l_acc, o_acc)
            if c == NC - 1:
                if t == len(items) - 1:
                    lraw_s[...] = l_acc
                    o_s[...] = o_acc
                else:
                    finalize(h, l_acc, o_acc)
        for t in range(DEPTH):
            sc_s[t] = ss[len(items) + t]
        return carry

    nxt = jnp.minimum(step + 1, NQ - 1)

    def slow_attention():
        prep(step)

        def head(h, carry):
            g = h // HPB

            def mx(c, m_acc):
                r0 = pl.multiple_of(c * TK, TK)
                s = _dot(k_s[g, pl.ds(r0, TK), :], qm_s[h])
                return jnp.maximum(m_acc, jnp.max(s, axis=0, keepdims=True))
            m = jax.lax.fori_loop(0, NC, mx, jnp.full((1, TQ), -jnp.inf, F32))

            def acc(c, lo):
                l_acc, o_acc = lo
                r0 = pl.multiple_of(c * TK, TK)
                s = _dot(k_s[g, pl.ds(r0, TK), :], qm_s[h])
                p = jnp.exp2(s - m)
                vt = vt_s[pl.ds(pl.multiple_of(h * DH, DH), DH), pl.ds(r0, TK)]
                return (l_acc + p.reshape(TK // 8, 8, TQ).sum(0), o_acc + _dot(vt, p.astype(BF16)))
            l_acc, o_acc = jax.lax.fori_loop(0, NC, acc, (jnp.zeros((8, TQ), F32), jnp.zeros((DH, TQ), F32)))
            finalize(h, l_acc, o_acc)
            lraw_s[...] = l_acc
            o_s[...] = o_acc
            return carry
        jax.lax.fori_loop(0, H, head, 0)
        for g in range(NG - 1):
            untranspose(g)
        for t in range(DEPTH):
            sc_s[t] = qk(H, 0, t)

    def attempt(state):
        a, _ = state

        @pl.when(a == 0)
        def _():
            jax.lax.fori_loop(0, NG, fast_body, 0)

        @pl.when(a == 1)
        def _():
            slow_attention()

        finalize(H - 1, lraw_s[...], o_s[...])
        untranspose(NG - 1)
        l_all = l_s[...]
        ok = jnp.logical_and(l_all >= L_LO, l_all <= L_HI)
        n_bad = jnp.sum(jnp.where(ok, 0.0, 1.0))

        nf = TQ // FC
        h1 = {}
        ln2 = {}
        act = {}
        for r in range(nf):
            rows = slice(r * FC, (r + 1) * FC)
            attn = None
            for g in range(NG):
                part = _dot(on_s[g, rows, :], wo_v[128 * g:128 * (g + 1), :])
                attn = part if attn is None else attn + part
            h1[r] = x_v[pl.ds(pl.multiple_of(q0 + r * FC, FC), FC), :].astype(F32) + attn
            ln2[r] = _ln(h1[r]).astype(BF16)
        prep(nxt)
        for r in range(nf):
            gate = _dot_nt(ln2[r], w1_v[...])
            up = _dot_nt(ln2[r], w3_v[...])
            act[r] = (gate * jax.nn.sigmoid(gate) * up).astype(BF16)
        for r in range(nf):
            y = _dot(act[r], w2_v[...])
            out_ref[0, r * FC:(r + 1) * FC, :] = (h1[r] + y).astype(out_ref.dtype)
        return a + 1, jnp.where(a == 0, (n_bad > 0.0).astype(jnp.int32), 0)

    jax.lax.while_loop(lambda s: s[0] < 1 + s[1], attempt, (jnp.int32(0), jnp.int32(0)))


@jax.jit
def pallas_sequential_preLN__softmax_full_mha__glu_gated_swiglu__prompt_kernel(
        A_x, A_wqkv, A_wo, B_x, B_w1, B_w3, B_w2):
    hbm = pl.BlockSpec(memory_space=pltpu.HBM)
    return pl.pallas_call(
        _kernel,
        grid=(NQ,),
        in_specs=[hbm] * 6,
        out_specs=pl.BlockSpec((1, TQ, D), lambda i: (0, i, 0)),
        out_shape=jax.ShapeDtypeStruct((1, S, D), BF16),
        scratch_shapes=[
            pltpu.VMEM((S, D), BF16),
            pltpu.VMEM((D, D), BF16),
            pltpu.VMEM((D, D), BF16),
            pltpu.VMEM((D, D), BF16),
            pltpu.VMEM((D, D), BF16),
            pltpu.VMEM((F, D), BF16),
            pltpu.VMEM((F, D), BF16),
            pltpu.VMEM((F, D), BF16),
            pltpu.VMEM((S, D), BF16),
            pltpu.VMEM((4, S, 128), BF16),
            pltpu.VMEM((D, S), BF16),
            pltpu.VMEM((D, S), BF16),
            pltpu.VMEM((H + 1, 128, TQ), BF16),
            pltpu.VMEM((D, TQ), BF16),
            pltpu.VMEM((NG, TQ, 128), BF16),
            pltpu.VMEM((H, S), F32),
            pltpu.VMEM((H, TQ), F32),
            pltpu.VMEM((DH, TQ), F32),
            pltpu.VMEM((8, TQ), F32),
            pltpu.VMEM((DEPTH, TK, TQ), F32),
            pltpu.SemaphoreType.DMA((NR + 7,)),
        ],
        compiler_params=pltpu.CompilerParams(
            dimension_semantics=("arbitrary",), vmem_limit_bytes=100 * 1024 * 1024),
        name="fused_block",
    )(A_x, A_wqkv, A_wo, B_w1.T, B_w3.T, B_w2)
```

```python
import math

import jax
import jax.numpy as jnp
import jax.experimental.pallas as pl
import jax.experimental.pallas.tpu as pltpu

S = 2048
D = 512
H = 32
DH = 16
F = 1376
TQ = 512
TK = 128
HPB = 8
DEPTH = 2
NQ = S // TQ
NC = S // TK
NG = H // HPB
RC = 512
NR = S // RC
FC = 256
EPS = 1e-5
QSCALE = (DH ** -0.5) * math.log2(math.e)
L_LO = 2.0 ** -80
L_HI = 2.0 ** 64

F32 = jnp.float32
BF16 = jnp.bfloat16


def _tree(op, xs):
    xs = list(xs)
    while len(xs) > 1:
        nxt = [op(xs[i], xs[i + 1]) for i in range(0, len(xs) - 1, 2)]
        if len(xs) % 2:
            nxt.append(xs[-1])
        xs = nxt
    return xs[0]


def _ln(x):
    m = jnp.mean(x, axis=-1, keepdims=True)
    xc = x - m
    v = jnp.mean(xc * xc, axis=-1, keepdims=True)
    return xc * jax.lax.rsqrt(v + EPS)


def _dot(a, b):
    return jnp.dot(a, b, preferred_element_type=F32)


def _dot_nt(a, b):
    return jax.lax.dot_general(a, b, (((1,), (1,)), ((), ())), preferred_element_type=F32)


def _kernel(x_hbm, wqkv_hbm, wo_hbm, w1_hbm, w3_hbm, w2_hbm, out_ref,
            x_v, wq_v, wk_v, wv_v, wo_v, w1_v, w3_v, w2_v,
            ln_s, k_s, vt_s, qt_s, qm_s, ot_s, on_s, m_s, l_s, o_s, lraw_s, sc_s, pc_s, lc_s, zs, sems):
    step = pl.program_id(0)

    def x_copy(c):
        return pltpu.make_async_copy(x_hbm.at[0, pl.ds(c * RC, RC), :], x_v.at[pl.ds(c * RC, RC), :], sems.at[c])

    def w_copy(i):
        src, dst = [(wqkv_hbm.at[:, pl.ds(D, D)], wk_v), (wqkv_hbm.at[:, pl.ds(2 * D, D)], wv_v),
                    (wqkv_hbm.at[:, pl.ds(0, D)], wq_v),
                    (wo_hbm, wo_v), (w1_hbm, w1_v), (w3_hbm, w3_v), (w2_hbm, w2_v)][i]
        return pltpu.make_async_copy(src, dst, sems.at[NR + i])

    def sel_matrix():
        head_of = jax.lax.broadcasted_iota(jnp.int32, (H, D), 1) // DH
        return (head_of == jax.lax.broadcasted_iota(jnp.int32, (H, D), 0)).astype(BF16)

    def qk(slot, g, c, z=0):
        return _dot(k_s[g, c * TK:(c + 1) * TK, :], qm_s[slot + z])

    def prep(tile):
        q0 = pl.multiple_of(tile * TQ, TQ)
        qt = qt_s[:, pl.ds(q0, TQ)]
        for h in range(H):
            j = h % 8
            qm_s[h, 16 * j:16 * j + 16, :] = qt[16 * h:16 * h + 16, :]
        q1 = pl.multiple_of(jnp.minimum(tile + 1, NQ - 1) * TQ, TQ)
        qm_s[H, 0:16, :] = qt_s[0:16, pl.ds(q1, TQ)]

    def softmax_num(s, m):
        p = jnp.exp2((s.reshape(TK // 8, 8, TQ) - m[None]).reshape(TK, TQ))
        ll = _tree(jnp.add, [p[8 * i:8 * i + 8] for i in range(TK // 8)])
        return p.astype(BF16), ll

    @pl.when(step == 0)
    def _prologue():
        for i in range(136):
            zs[i] = 0
        x_copy(0).start()
        w_copy(0).start()
        for c in range(1, NR):
            x_copy(c).start()
        w_copy(1).start()
        w_copy(2).start()
        qm_s[...] = jnp.zeros(qm_s.shape, qm_s.dtype)
        ot_s[...] = jnp.zeros(ot_s.shape, ot_s.dtype)
        o_s[...] = jnp.zeros(o_s.shape, F32)
        lraw_s[...] = jnp.ones(lraw_s.shape, F32)

        def ln_chunk(c):
            rows = slice(c * RC, (c + 1) * RC)
            ln_s[rows, :] = _ln(x_v[rows, :].astype(F32)).astype(BF16)

        def k_chunk(c):
            rows = slice(c * RC, (c + 1) * RC)
            k = _dot(ln_s[rows, :], wk_v[...]).astype(BF16)
            for g in range(4):
                k_s[g, rows, :] = k[:, 128 * g:128 * (g + 1)]
            kf = k.astype(F32)
            return jnp.max((kf * kf).reshape(RC // 8, 8, D), axis=0)

        x_copy(0).wait()
        ln_chunk(0)
        w_copy(0).wait()
        x_copy(1).wait()
        ksq = [k_chunk(0)]
        ln_chunk(1)
        x_copy(2).wait()
        ksq.append(k_chunk(1))
        ln_chunk(2)
        x_copy(3).wait()
        w_copy(1).wait()
        w_copy(2).wait()
        for i in range(3, 7):
            w_copy(i).start()
        ksq.append(k_chunk(2))
        ln_chunk(3)
        wvt = wv_v[...].T
        wqt = wq_v[...].T
        ksq.append(k_chunk(3))
        cmax = jnp.maximum(jnp.maximum(ksq[0], ksq[1]), jnp.maximum(ksq[2], ksq[3]))
        cmax = jnp.broadcast_to(jnp.max(cmax, axis=0, keepdims=True), (128, D)).astype(BF16)
        kb2 = _dot_nt(sel_matrix(), cmax)
        for c in range(NR):
            rows = slice(c * RC, (c + 1) * RC)
            q = (_dot_nt(wqt, ln_s[rows, :]) * QSCALE).astype(BF16)
            qt_s[:, rows] = q
            qf = q.astype(F32)
            qsq = qf * qf
            for h in range(H):
                t = qsq[16 * h:16 * h + 8] + qsq[16 * h + 8:16 * h + 16]
                for sh in (4, 2, 1):
                    t = t + pltpu.roll(t, sh, 0)
                kb = jnp.concatenate([kb2[h:h + 1, :]] * (RC // 128), axis=1)
                t = t * kb + 1e-30
                m_s[h, :, rows] = t * jax.lax.rsqrt(t) * 1.02
        prep(0)
        for c in range(NR):
            rows = slice(c * RC, (c + 1) * RC)
            vt_s[:, rows] = _dot_nt(wvt, ln_s[rows, :]).astype(BF16)
            if c == 1:
                s_init = [qk(0, 0, t) for t in range(DEPTH)]
        pb, ll = softmax_num(s_init[0], m_s[0, :, 0:TQ])
        pc_s[...] = pb
        lc_s[...] = ll
        sc_s[...] = s_init[1]
        for i in range(3, 7):
            w_copy(i).wait()

    q0 = pl.multiple_of(step * TQ, TQ)
    nxt = jnp.minimum(step + 1, NQ - 1)
    q_next = pl.multiple_of(nxt * TQ, TQ)

    def pv(h, c, pb, ll, l_acc, o_acc):
        l_acc = ll if l_acc is None else l_acc + ll
        vt = vt_s[pl.ds(pl.multiple_of(h * DH, DH), DH), c * TK:(c + 1) * TK]
        oo = _dot(vt, pb)
        o_acc = oo if o_acc is None else o_acc + oo
        return l_acc, o_acc

    def load_m(h, qoff):
        return m_s[h, :, pl.ds(qoff, TQ)]

    def finalize(h, l_acc, o_acc, after=None):
        l = l_acc.sum(0, keepdims=True)
        if after is not None:
            z = on_s[after, 0:16, :].astype(F32)[0:1, :] * 0.0
            l = l + jnp.concatenate([z] * (TQ // 128), axis=1)
        l_s[pl.ds(h, 1), :] = l
        ot_s[pl.ds(pl.multiple_of(h * DH, DH), DH), :] = (o_acc * pl.reciprocal(l, approx=False)).astype(BF16)

    def untranspose(g):
        on_s[g] = ot_s[pl.ds(pl.multiple_of(g * 128, 128), 128), :].T

    def carry_out(s0, s1, h, qoff):
        pb, ll = softmax_num(s0, load_m(h, qoff))
        pc_s[...] = pb
        lc_s[...] = ll
        sc_s[...] = s1

    def fast_body(i, carry):
        finalize(jnp.maximum(i * HPB - 1, 0), lraw_s[...], o_s[...])
        untranspose(jnp.maximum(i - 1, 0))
        items = [(i * HPB + j, i, c) for j in range(HPB) for c in range(NC)]
        last = i == NG - 1
        nslot = jnp.where(last, H, (i + 1) * HPB)
        ng = jnp.where(last, 0, i + 1)
        items_all = items + [(nslot, ng, c) for c in range(DEPTH)]
        ss = {1: sc_s[...]}
        m = l_acc = o_acc = None
        for t, (h, g, c) in enumerate(items):
            ss[t + DEPTH] = qk(*items_all[t + DEPTH], z=zs[t])
            if c == 0:
                m = load_m(h, q0)
                l_acc = o_acc = None
            if t == 0:
                pb, ll = pc_s[...], lc_s[...]
            else:
                pb, ll = softmax_num(ss.pop(t), m)
            l_acc, o_acc = pv(h, c, pb, ll, l_acc, o_acc)
            if c == NC - 1:
                if t == len(items) - 1:
                    lraw_s[...] = l_acc
                    o_s[...] = o_acc
                else:
                    finalize(h, l_acc, o_acc, after=jnp.maximum(i - 1, 0) if t < NC else None)
        n = len(items)
        carry_out(ss[n], ss[n + 1], jnp.where(last, 0, (i + 1) * HPB), jnp.where(last, q_next, q0))
        return carry


    def slow_attention():
        prep(step)

        def head(h, carry):
            g = h // HPB

            def mx(c, m_acc):
                r0 = pl.multiple_of(c * TK, TK)
                s = _dot(k_s[g, pl.ds(r0, TK), :], qm_s[h])
                return jnp.maximum(m_acc, jnp.max(s, axis=0, keepdims=True))
            m = jax.lax.fori_loop(0, NC, mx, jnp.full((1, TQ), -jnp.inf, F32))

            def acc(c, lo):
                l_acc, o_acc = lo
                r0 = pl.multiple_of(c * TK, TK)
                s = _dot(k_s[g, pl.ds(r0, TK), :], qm_s[h])
                p = jnp.exp2(s - m)
                vt = vt_s[pl.ds(pl.multiple_of(h * DH, DH), DH), pl.ds(r0, TK)]
                return (l_acc + p.reshape(TK // 8, 8, TQ).sum(0), o_acc + _dot(vt, p.astype(BF16)))
            l_acc, o_acc = jax.lax.fori_loop(0, NC, acc, (jnp.zeros((8, TQ), F32), jnp.zeros((DH, TQ), F32)))
            finalize(h, l_acc, o_acc)
            lraw_s[...] = l_acc
            o_s[...] = o_acc
            return carry
        jax.lax.fori_loop(0, H, head, 0)
        for g in range(NG - 1):
            untranspose(g)
        carry_out(qk(H, 0, 0), qk(H, 0, 1), 0, q_next)

    def attempt(state):
        a, _ = state

        @pl.when(a == 0)
        def _():
            jax.lax.fori_loop(0, NG, fast_body, 0)

        @pl.when(a == 1)
        def _():
            slow_attention()

        finalize(H - 1, lraw_s[...], o_s[...])
        untranspose(NG - 1)
        l_all = l_s[...]
        ok = jnp.logical_and(l_all >= L_LO, l_all <= L_HI)
        n_bad = jnp.sum(jnp.where(ok, 0.0, 1.0))

        nf = TQ // FC
        h1 = {}
        ln2 = {}
        act = {}
        for r in range(nf):
            rows = slice(r * FC, (r + 1) * FC)
            attn = None
            for g in range(NG):
                part = _dot(on_s[g, rows, :], wo_v[128 * g:128 * (g + 1), :])
                attn = part if attn is None else attn + part
            h1[r] = x_v[pl.ds(pl.multiple_of(q0 + r * FC, FC), FC), :].astype(F32) + attn
            ln2[r] = _ln(h1[r]).astype(BF16)
        prep(nxt)
        for r in range(nf):
            gate = _dot_nt(ln2[r], w1_v[...])
            up = _dot_nt(ln2[r], w3_v[...])
            act[r] = (gate * jax.nn.sigmoid(gate) * up).astype(BF16)
        for r in range(nf):
            y = _dot(act[r], w2_v[...])
            out_ref[0, r * FC:(r + 1) * FC, :] = (h1[r] + y).astype(out_ref.dtype)
        return a + 1, jnp.where(a == 0, (n_bad > 0.0).astype(jnp.int32), 0)

    jax.lax.while_loop(lambda s: s[0] < 1 + s[1], attempt, (jnp.int32(0), jnp.int32(0)))


@jax.jit
def pallas_sequential_preLN__softmax_full_mha__glu_gated_swiglu__prompt_kernel(
        A_x, A_wqkv, A_wo, B_x, B_w1, B_w3, B_w2):
    hbm = pl.BlockSpec(memory_space=pltpu.HBM)
    return pl.pallas_call(
        _kernel,
        grid=(NQ,),
        in_specs=[hbm] * 6,
        out_specs=pl.BlockSpec((1, TQ, D), lambda i: (0, i, 0)),
        out_shape=jax.ShapeDtypeStruct((1, S, D), BF16),
        scratch_shapes=[
            pltpu.VMEM((S, D), BF16),
            pltpu.VMEM((D, D), BF16),
            pltpu.VMEM((D, D), BF16),
            pltpu.VMEM((D, D), BF16),
            pltpu.VMEM((D, D), BF16),
            pltpu.VMEM((F, D), BF16),
            pltpu.VMEM((F, D), BF16),
            pltpu.VMEM((F, D), BF16),
            pltpu.VMEM((S, D), BF16),
            pltpu.VMEM((4, S, 128), BF16),
            pltpu.VMEM((D, S), BF16),
            pltpu.VMEM((D, S), BF16),
            pltpu.VMEM((H + 1, 128, TQ), BF16),
            pltpu.VMEM((D, TQ), BF16),
            pltpu.VMEM((NG, TQ, 128), BF16),
            pltpu.VMEM((H, 8, S), F32),
            pltpu.VMEM((H, TQ), F32),
            pltpu.VMEM((DH, TQ), F32),
            pltpu.VMEM((8, TQ), F32),
            pltpu.VMEM((TK, TQ), F32),
            pltpu.VMEM((TK, TQ), BF16),
            pltpu.VMEM((8, TQ), F32),
            pltpu.SMEM((136,), jnp.int32),
            pltpu.SemaphoreType.DMA((NR + 7,)),
        ],
        compiler_params=pltpu.CompilerParams(
            dimension_semantics=("arbitrary",), vmem_limit_bytes=100 * 1024 * 1024),
        name="fused_block",
    )(A_x, A_wqkv, A_wo, B_w1.T, B_w3.T, B_w2)
```

```python
import math

import jax
import jax.numpy as jnp
import jax.experimental.pallas as pl
import jax.experimental.pallas.tpu as pltpu

S = 2048
D = 512
H = 32
DH = 16
F = 1376
TQ = 512
TK = 128
HPB = 8
DEPTH = 2
NQ = S // TQ
NC = S // TK
NG = H // HPB
RC = 512
NR = S // RC
FC = 256
OC = 128
EPS = 1e-5
QSCALE = (DH ** -0.5) * math.log2(math.e)
L_LO = 2.0 ** -80
L_HI = 2.0 ** 64

F32 = jnp.float32
BF16 = jnp.bfloat16


def _tree(op, xs):
    xs = list(xs)
    while len(xs) > 1:
        nxt = [op(xs[i], xs[i + 1]) for i in range(0, len(xs) - 1, 2)]
        if len(xs) % 2:
            nxt.append(xs[-1])
        xs = nxt
    return xs[0]


def _ln(x):
    m = jnp.mean(x, axis=-1, keepdims=True)
    xc = x - m
    v = jnp.mean(xc * xc, axis=-1, keepdims=True)
    return xc * jax.lax.rsqrt(v + EPS)


def _dot(a, b):
    return jnp.dot(a, b, preferred_element_type=F32)


def _dot_nt(a, b):
    return jax.lax.dot_general(a, b, (((1,), (1,)), ((), ())), preferred_element_type=F32)


def _kernel(x_hbm, wqkv_hbm, wo_hbm, w1_hbm, w3_hbm, w2_hbm, out_hbm,
            x_v, wq_v, wk_v, wv_v, wo_v, w1_v, w3_v, w2_v,
            ln_s, k_s, vt_s, qt_s, qm_s, ot_s, on_s, m_s, l_s, o_s, lraw_s, sc_s, pc_s, lc_s, out_v, zs, sems, osems):
    step = pl.program_id(0)

    def x_copy(c):
        return pltpu.make_async_copy(x_hbm.at[0, pl.ds(c * RC, RC), :], x_v.at[pl.ds(c * RC, RC), :], sems.at[c])

    def w_copy(i):
        src, dst = [(wqkv_hbm.at[:, pl.ds(D, D)], wk_v), (wqkv_hbm.at[:, pl.ds(2 * D, D)], wv_v),
                    (wqkv_hbm.at[:, pl.ds(0, D)], wq_v),
                    (wo_hbm, wo_v), (w1_hbm, w1_v), (w3_hbm, w3_v), (w2_hbm, w2_v)][i]
        return pltpu.make_async_copy(src, dst, sems.at[NR + i])

    def out_copy(r, tile):
        return pltpu.make_async_copy(out_v.at[pl.ds(r * OC, OC), :],
                                     out_hbm.at[0, pl.ds(pl.multiple_of(tile * TQ + r * OC, OC), OC), :], osems.at[r])

    def sel_matrix():
        head_of = jax.lax.broadcasted_iota(jnp.int32, (H, D), 1) // DH
        return (head_of == jax.lax.broadcasted_iota(jnp.int32, (H, D), 0)).astype(F32)

    def qk(slot, g, c, z=0):
        return _dot(k_s[g, c * TK:(c + 1) * TK, :], qm_s[slot + z])

    def prep(tile):
        q0 = pl.multiple_of(tile * TQ, TQ)
        qt = qt_s[:, pl.ds(q0, TQ)]
        for h in range(H):
            j = h % 8
            qm_s[h, 16 * j:16 * j + 16, :] = qt[16 * h:16 * h + 16, :]
        q1 = pl.multiple_of(jnp.minimum(tile + 1, NQ - 1) * TQ, TQ)
        qm_s[H, 0:16, :] = qt_s[0:16, pl.ds(q1, TQ)]

    def softmax_num(s, m):
        p = jnp.exp2((s.reshape(TK // 8, 8, TQ) - m[None]).reshape(TK, TQ))
        ll = _tree(jnp.add, [p[8 * i:8 * i + 8] for i in range(TK // 8)])
        return p.astype(BF16), ll

    @pl.when(step == 0)
    def _prologue():
        for i in range(136):
            zs[i] = 0
        x_copy(0).start()
        w_copy(0).start()
        for c in range(1, NR):
            x_copy(c).start()
        w_copy(1).start()
        w_copy(2).start()
        qm_s[...] = jnp.zeros(qm_s.shape, qm_s.dtype)
        ot_s[...] = jnp.zeros(ot_s.shape, ot_s.dtype)
        o_s[...] = jnp.zeros(o_s.shape, F32)
        lraw_s[...] = jnp.ones(lraw_s.shape, F32)

        def ln_chunk(c):
            rows = slice(c * RC, (c + 1) * RC)
            ln_s[rows, :] = _ln(x_v[rows, :].astype(F32)).astype(BF16)

        def k_chunk(c):
            rows = slice(c * RC, (c + 1) * RC)
            k = _dot(ln_s[rows, :], wk_v[...]).astype(BF16)
            for g in range(4):
                k_s[g, rows, :] = k[:, 128 * g:128 * (g + 1)]
            return jnp.max(jnp.abs(k.astype(F32)).reshape(RC // 8, 8, D), axis=0)

        x_copy(0).wait()
        ln_chunk(0)
        w_copy(0).wait()
        x_copy(1).wait()
        ksq = [k_chunk(0)]
        ln_chunk(1)
        x_copy(2).wait()
        ksq.append(k_chunk(1))
        ln_chunk(2)
        x_copy(3).wait()
        w_copy(1).wait()
        w_copy(2).wait()
        for i in range(3, 7):
            w_copy(i).start()
        ksq.append(k_chunk(2))
        ln_chunk(3)
        wvt = wv_v[...].T
        wqt = wq_v[...].T
        ksq.append(k_chunk(3))
        kabs = jnp.maximum(jnp.maximum(ksq[0], ksq[1]), jnp.maximum(ksq[2], ksq[3]))
        kabs = jnp.max(kabs, axis=0, keepdims=True) * 1.02
        bound = (sel_matrix() * kabs).astype(BF16)
        for c in range(NR):
            rows = slice(c * RC, (c + 1) * RC)
            qt_s[:, rows] = (_dot_nt(wqt, ln_s[rows, :]) * QSCALE).astype(BF16)
        prep(0)

        def stabiliser(c):
            rows = slice(c * RC, (c + 1) * RC)
            qabs = pltpu.bitcast(pltpu.bitcast(qt_s[:, rows], jnp.uint32) & jnp.uint32(0x7FFF7FFF), BF16)
            mm = _dot(bound, qabs)
            for h in range(H):
                m_s[h, :, rows] = jnp.broadcast_to(mm[h:h + 1, :], (8, RC))

        for c in range(NR):
            rows = slice(c * RC, (c + 1) * RC)
            vt_s[:, rows] = _dot_nt(wvt, ln_s[rows, :]).astype(BF16)
            stabiliser(c)
            if c == 1:
                s_init = [qk(0, 0, t) for t in range(DEPTH)]
        pb, ll = softmax_num(s_init[0], m_s[0, :, 0:TQ])
        pc_s[...] = pb
        lc_s[...] = ll
        sc_s[...] = s_init[1]
        for i in range(3, 7):
            w_copy(i).wait()

    q0 = pl.multiple_of(step * TQ, TQ)
    nxt = jnp.minimum(step + 1, NQ - 1)
    q_next = pl.multiple_of(nxt * TQ, TQ)

    def pv(h, c, pb, ll, l_acc, o_acc):
        l_acc = ll if l_acc is None else l_acc + ll
        vt = vt_s[pl.ds(pl.multiple_of(h * DH, DH), DH), c * TK:(c + 1) * TK]
        oo = _dot(vt, pb)
        o_acc = oo if o_acc is None else o_acc + oo
        return l_acc, o_acc

    def load_m(h, qoff):
        return m_s[h, :, pl.ds(qoff, TQ)]

    def finalize(h, l_acc, o_acc, after=None):
        l = l_acc.sum(0, keepdims=True)
        if after is not None:
            z = on_s[after, 0:16, :].astype(F32)[0:1, :] * 0.0
            l = l + jnp.concatenate([z] * (TQ // 128), axis=1)
        l_s[pl.ds(h, 1), :] = l
        ot_s[pl.ds(pl.multiple_of(h * DH, DH), DH), :] = (o_acc * pl.reciprocal(l, approx=False)).astype(BF16)

    def untranspose(g):
        on_s[g] = ot_s[pl.ds(pl.multiple_of(g * 128, 128), 128), :].T

    def carry_out(s0, s1, h, qoff):
        pb, ll = softmax_num(s0, load_m(h, qoff))
        pc_s[...] = pb
        lc_s[...] = ll
        sc_s[...] = s1

    def fast_body(i, carry):
        finalize(jnp.maximum(i * HPB - 1, 0), lraw_s[...], o_s[...])
        untranspose(jnp.maximum(i - 1, 0))
        items = [(i * HPB + j, i, c) for j in range(HPB) for c in range(NC)]
        last = i == NG - 1
        nslot = jnp.where(last, H, (i + 1) * HPB)
        ng = jnp.where(last, 0, i + 1)
        items_all = items + [(nslot, ng, c) for c in range(DEPTH)]
        ss = {1: sc_s[...]}
        m = l_acc = o_acc = None
        for t, (h, g, c) in enumerate(items):
            ss[t + DEPTH] = qk(*items_all[t + DEPTH], z=zs[t])
            if c == 0:
                m = load_m(h, q0)
                l_acc = o_acc = None
            if t == 0:
                pb, ll = pc_s[...], lc_s[...]
            else:
                pb, ll = softmax_num(ss.pop(t), m)
            l_acc, o_acc = pv(h, c, pb, ll, l_acc, o_acc)
            if c == NC - 1:
                if t == len(items) - 1:
                    lraw_s[...] = l_acc
                    o_s[...] = o_acc
                else:
                    finalize(h, l_acc, o_acc, after=jnp.maximum(i - 1, 0) if t < NC else None)
        n = len(items)
        carry_out(ss[n], ss[n + 1], jnp.where(last, 0, (i + 1) * HPB), jnp.where(last, q_next, q0))
        return carry


    def slow_attention():
        prep(step)

        def head(h, carry):
            g = h // HPB

            def mx(c, m_acc):
                r0 = pl.multiple_of(c * TK, TK)
                s = _dot(k_s[g, pl.ds(r0, TK), :], qm_s[h])
                return jnp.maximum(m_acc, jnp.max(s, axis=0, keepdims=True))
            m = jax.lax.fori_loop(0, NC, mx, jnp.full((1, TQ), -jnp.inf, F32))

            def acc(c, lo):
                l_acc, o_acc = lo
                r0 = pl.multiple_of(c * TK, TK)
                s = _dot(k_s[g, pl.ds(r0, TK), :], qm_s[h])
                p = jnp.exp2(s - m)
                vt = vt_s[pl.ds(pl.multiple_of(h * DH, DH), DH), pl.ds(r0, TK)]
                return (l_acc + p.reshape(TK // 8, 8, TQ).sum(0), o_acc + _dot(vt, p.astype(BF16)))
            l_acc, o_acc = jax.lax.fori_loop(0, NC, acc, (jnp.zeros((8, TQ), F32), jnp.zeros((DH, TQ), F32)))
            finalize(h, l_acc, o_acc)
            lraw_s[...] = l_acc
            o_s[...] = o_acc
            return carry
        jax.lax.fori_loop(0, H, head, 0)
        for g in range(NG - 1):
            untranspose(g)
        carry_out(qk(H, 0, 0), qk(H, 0, 1), 0, q_next)

    def attempt(state):
        a, _ = state

        @pl.when(a == 0)
        def _():
            jax.lax.fori_loop(0, NG, fast_body, 0)

        @pl.when(a == 1)
        def _():
            slow_attention()

        @pl.when(jnp.logical_or(step > 0, a > 0))
        def _():
            prev = jnp.where(a > 0, step, jnp.maximum(step - 1, 0))
            for r in range(TQ // OC):
                out_copy(r, prev).wait()

        finalize(H - 1, lraw_s[...], o_s[...])
        untranspose(NG - 1)
        l_all = l_s[...]
        ok = jnp.logical_and(l_all >= L_LO, l_all <= L_HI)
        n_bad = jnp.sum(jnp.where(ok, 0.0, 1.0))

        nf = TQ // FC
        h1 = {}
        ln2 = {}
        act = {}
        for r in range(nf):
            rows = slice(r * FC, (r + 1) * FC)
            attn = None
            for g in range(NG):
                part = _dot(on_s[g, rows, :], wo_v[128 * g:128 * (g + 1), :])
                attn = part if attn is None else attn + part
            h1[r] = x_v[pl.ds(pl.multiple_of(q0 + r * FC, FC), FC), :].astype(F32) + attn
            ln2[r] = _ln(h1[r]).astype(BF16)
        prep(nxt)
        for r in range(nf):
            gate = _dot_nt(ln2[r], w1_v[...])
            up = _dot_nt(ln2[r], w3_v[...])
            act[r] = (gate * jax.nn.sigmoid(gate) * up).astype(BF16)
        for r in range(nf):
            for u in range(FC // OC):
                y = _dot(act[r][u * OC:(u + 1) * OC], w2_v[...])
                k = r * (FC // OC) + u
                out_v[k * OC:(k + 1) * OC, :] = (h1[r][u * OC:(u + 1) * OC] + y).astype(BF16)
                out_copy(k, step).start()
        return a + 1, jnp.where(a == 0, (n_bad > 0.0).astype(jnp.int32), 0)

    jax.lax.while_loop(lambda s: s[0] < 1 + s[1], attempt, (jnp.int32(0), jnp.int32(0)))

    @pl.when(step == NQ - 1)
    def _():
        for r in range(TQ // OC):
            out_copy(r, step).wait()


@jax.jit
def pallas_sequential_preLN__softmax_full_mha__glu_gated_swiglu__prompt_kernel(
        A_x, A_wqkv, A_wo, B_x, B_w1, B_w3, B_w2):
    hbm = pl.BlockSpec(memory_space=pltpu.HBM)
    return pl.pallas_call(
        _kernel,
        grid=(NQ,),
        in_specs=[hbm] * 6,
        out_specs=hbm,
        out_shape=jax.ShapeDtypeStruct((1, S, D), BF16),
        scratch_shapes=[
            pltpu.VMEM((S, D), BF16),
            pltpu.VMEM((D, D), BF16),
            pltpu.VMEM((D, D), BF16),
            pltpu.VMEM((D, D), BF16),
            pltpu.VMEM((D, D), BF16),
            pltpu.VMEM((F, D), BF16),
            pltpu.VMEM((F, D), BF16),
            pltpu.VMEM((F, D), BF16),
            pltpu.VMEM((S, D), BF16),
            pltpu.VMEM((4, S, 128), BF16),
            pltpu.VMEM((D, S), BF16),
            pltpu.VMEM((D, S), BF16),
            pltpu.VMEM((H + 1, 128, TQ), BF16),
            pltpu.VMEM((D, TQ), BF16),
            pltpu.VMEM((NG, TQ, 128), BF16),
            pltpu.VMEM((H, 8, S), F32),
            pltpu.VMEM((H, TQ), F32),
            pltpu.VMEM((DH, TQ), F32),
            pltpu.VMEM((8, TQ), F32),
            pltpu.VMEM((TK, TQ), F32),
            pltpu.VMEM((TK, TQ), BF16),
            pltpu.VMEM((8, TQ), F32),
            pltpu.VMEM((TQ, D), BF16),
            pltpu.SMEM((136,), jnp.int32),
            pltpu.SemaphoreType.DMA((NR + 7,)),
            pltpu.SemaphoreType.DMA((TQ // OC,)),
        ],
        compiler_params=pltpu.CompilerParams(
            dimension_semantics=("arbitrary",), vmem_limit_bytes=100 * 1024 * 1024),
        name="fused_block",
    )(A_x, A_wqkv, A_wo, B_w1.T, B_w3.T, B_w2)
```

```python
import math

import jax
import jax.numpy as jnp
import jax.experimental.pallas as pl
import jax.experimental.pallas.tpu as pltpu

S = 2048
D = 512
H = 32
DH = 16
F = 1376
TQ = 512
TK = 128
HPB = 8
DEPTH = 2
NQ = S // TQ
NC = S // TK
NG = H // HPB
RC = 512
NR = S // RC
XB = (0, 256, 512, 1024, 1536, 2048)
NX = len(XB) - 1
FC = 128
OC = 128
NO = TQ // OC
EPS = 1e-5
QSCALE = (DH ** -0.5) * math.log2(math.e)
L_LO = 2.0 ** -60
L_HI = 2.0 ** 64

F32 = jnp.float32
BF16 = jnp.bfloat16


def _tree(op, xs):
    xs = list(xs)
    while len(xs) > 1:
        nxt = [op(xs[i], xs[i + 1]) for i in range(0, len(xs) - 1, 2)]
        if len(xs) % 2:
            nxt.append(xs[-1])
        xs = nxt
    return xs[0]


def _ln(x):
    m = jnp.mean(x, axis=-1, keepdims=True)
    xc = x - m
    v = jnp.mean(xc * xc, axis=-1, keepdims=True)
    return xc * jax.lax.rsqrt(v + EPS)


def _dot(a, b):
    return jnp.dot(a, b, preferred_element_type=F32)


def _dot_nt(a, b):
    return jax.lax.dot_general(a, b, (((1,), (1,)), ((), ())), preferred_element_type=F32)


def _kernel(x_hbm, wqkv_hbm, wo_hbm, w1_hbm, w3_hbm, w2_hbm, out_hbm,
            x_v, wq_v, wk_v, wv_v, wo_v, w1_v, w3_v, w2_v,
            ln_s, k_s, vt_s, qt_s, qm_s, ot_s, on_s, m_s, l_s, o_s, lraw_s, sc_s, pc_s, lc_s,
            out_v, zs, sems, osems):
    step = pl.program_id(0)
    q0 = pl.multiple_of(step * TQ, TQ)
    nxt = jnp.minimum(step + 1, NQ - 1)
    q_next = pl.multiple_of(nxt * TQ, TQ)

    def x_copy(c):
        n = XB[c + 1] - XB[c]
        return pltpu.make_async_copy(x_hbm.at[0, pl.ds(XB[c], n), :], x_v.at[pl.ds(XB[c], n), :], sems.at[c])

    def w_copy(i):
        src, dst = [(wqkv_hbm.at[:, pl.ds(D, D)], wk_v), (wqkv_hbm.at[:, pl.ds(2 * D, D)], wv_v),
                    (wqkv_hbm.at[:, pl.ds(0, D)], wq_v),
                    (wo_hbm, wo_v), (w1_hbm, w1_v), (w3_hbm, w3_v), (w2_hbm, w2_v)][i]
        return pltpu.make_async_copy(src, dst, sems.at[NX + i])

    def out_copy(r, tile):
        return pltpu.make_async_copy(out_v.at[pl.ds(r * OC, OC), :],
                                     out_hbm.at[0, pl.ds(pl.multiple_of(tile * TQ + r * OC, OC), OC), :],
                                     osems.at[r])

    def qk(slot, g, c, z=0):
        return _dot(k_s[g, c * TK:(c + 1) * TK, :], qm_s[slot + z])

    def prep(tile):
        qt = qt_s[:, pl.ds(pl.multiple_of(tile * TQ, TQ), TQ)]
        for h in range(H):
            j = h % 8
            qm_s[h, 16 * j:16 * j + 16, :] = qt[16 * h:16 * h + 16, :]
        q1 = pl.multiple_of(jnp.minimum(tile + 1, NQ - 1) * TQ, TQ)
        qm_s[H, 0:16, :] = qt_s[0:16, pl.ds(q1, TQ)]

    def softmax_num(s, m):
        p = jnp.exp2((s.reshape(TK // 8, 8, TQ) - m[None]).reshape(TK, TQ))
        ll = _tree(jnp.add, [p[8 * i:8 * i + 8] for i in range(TK // 8)])
        return p.astype(BF16), ll

    def carry_out(s0, s1, m):
        pb, ll = softmax_num(s0, m)
        pc_s[...] = pb
        lc_s[...] = ll
        sc_s[...] = s1

    @pl.when(step == 0)
    def _prologue():
        for i in range(HPB * NC):
            zs[i] = 0
        x_copy(0).start()
        w_copy(0).start()
        for c in range(1, NX):
            x_copy(c).start()
        w_copy(1).start()
        w_copy(2).start()
        qm_s[...] = jnp.zeros(qm_s.shape, qm_s.dtype)
        ot_s[...] = jnp.zeros(ot_s.shape, ot_s.dtype)
        o_s[...] = jnp.zeros(o_s.shape, F32)
        lraw_s[...] = jnp.ones(lraw_s.shape, F32)

        def ln_chunk(c):
            rows = slice(XB[c], XB[c + 1])
            ln_s[rows, :] = _ln(x_v[rows, :].astype(F32)).astype(BF16)

        def k_chunk(c):
            rows = slice(XB[c], XB[c + 1])
            k = _dot(ln_s[rows, :], wk_v[...]).astype(BF16)
            for g in range(4):
                k_s[g, rows, :] = k[:, 128 * g:128 * (g + 1)]
            return jnp.max(jnp.abs(k.astype(F32)).reshape(-1, 8, D), axis=0)

        x_copy(0).wait()
        ln_chunk(0)
        w_copy(0).wait()
        kabs = None
        for c in range(NX - 1):
            x_copy(c + 1).wait()
            if c == NX - 2:
                w_copy(1).wait()
                w_copy(2).wait()
                for i in range(3, 7):
                    w_copy(i).start()
            ka = k_chunk(c)
            kabs = ka if kabs is None else jnp.maximum(kabs, ka)
            ln_chunk(c + 1)
        wvt = wv_v[...].T
        wqt = wq_v[...].T
        kabs = jnp.maximum(kabs, k_chunk(NX - 1))
        kabs = jnp.max(kabs, axis=0, keepdims=True) * 1.02
        head_of = jax.lax.broadcasted_iota(jnp.int32, (H, D), 1) // DH
        sel = (head_of == jax.lax.broadcasted_iota(jnp.int32, (H, D), 0)).astype(F32)
        bound = (sel * kabs).astype(BF16)
        for c in range(NR):
            rows = slice(c * RC, (c + 1) * RC)
            qt_s[:, rows] = (_dot_nt(wqt, ln_s[rows, :]) * QSCALE).astype(BF16)
        prep(0)
        for c in range(NR):
            rows = slice(c * RC, (c + 1) * RC)
            vt_s[:, rows] = _dot_nt(wvt, ln_s[rows, :]).astype(BF16)
            qabs = jnp.abs(qt_s[:, rows].astype(F32)).astype(BF16)
            mm = _dot(bound, qabs)
            for h in range(H):
                m_s[h, :, rows] = jnp.broadcast_to(mm[h:h + 1, :], (8, RC))
            if c == 1:
                s_init = [qk(0, 0, t) for t in range(DEPTH)]
        carry_out(s_init[0], s_init[1], m_s[0, :, 0:TQ])
        for i in range(3, 7):
            w_copy(i).wait()

    def pv(h, c, pb, ll, l_acc, o_acc):
        l_acc = ll if l_acc is None else l_acc + ll
        vt = vt_s[pl.ds(pl.multiple_of(h * DH, DH), DH), c * TK:(c + 1) * TK]
        oo = _dot(vt, pb)
        o_acc = oo if o_acc is None else o_acc + oo
        return l_acc, o_acc

    def load_m(h, qoff):
        return m_s[h, :, pl.ds(qoff, TQ)]

    def finalize(h, l_acc, o_acc, after=None):
        l = l_acc.sum(0, keepdims=True)
        if after is not None:
            z = on_s[after, 0:16, :].astype(F32)[0:1, :] * 0.0
            l = l + jnp.concatenate([z] * (TQ // 128), axis=1)
        l_s[pl.ds(h, 1), :] = l
        ot_s[pl.ds(pl.multiple_of(h * DH, DH), DH), :] = (o_acc * pl.reciprocal(l, approx=False)).astype(BF16)

    def untranspose(g):
        on_s[g] = ot_s[pl.ds(pl.multiple_of(g * 128, 128), 128), :].T

    def fast_body(i, carry):
        finalize(jnp.maximum(i * HPB - 1, 0), lraw_s[...], o_s[...])
        untranspose(jnp.maximum(i - 1, 0))
        items = [(i * HPB + j, i, c) for j in range(HPB) for c in range(NC)]
        last = i == NG - 1
        nslot = jnp.where(last, H, (i + 1) * HPB)
        ng = jnp.where(last, 0, i + 1)
        items_all = items + [(nslot, ng, c) for c in range(DEPTH)]
        ss = {1: sc_s[...]}
        m = l_acc = o_acc = None
        for t, (h, g, c) in enumerate(items):
            ss[t + DEPTH] = qk(*items_all[t + DEPTH], z=zs[t])
            if c == 0:
                m = load_m(h, q0)
                l_acc = o_acc = None
            if t == 0:
                pb, ll = pc_s[...], lc_s[...]
            else:
                pb, ll = softmax_num(ss.pop(t), m)
            l_acc, o_acc = pv(h, c, pb, ll, l_acc, o_acc)
            if c == NC - 1:
                if t == len(items) - 1:
                    lraw_s[...] = l_acc
                    o_s[...] = o_acc
                else:
                    finalize(h, l_acc, o_acc, after=jnp.maximum(i - 1, 0) if t < NC else None)
        n = len(items)
        carry_out(ss[n], ss[n + 1], load_m(jnp.where(last, 0, (i + 1) * HPB), jnp.where(last, q_next, q0)))
        return carry

    def slow_attention():
        prep(step)

        def head(h, carry):
            g = h // HPB

            def mx(c, m_acc):
                r0 = pl.multiple_of(c * TK, TK)
                s = _dot(k_s[g, pl.ds(r0, TK), :], qm_s[h])
                return jnp.maximum(m_acc, jnp.max(s, axis=0, keepdims=True))
            m = jax.lax.fori_loop(0, NC, mx, jnp.full((1, TQ), -jnp.inf, F32))

            def acc(c, lo):
                l_acc, o_acc = lo
                r0 = pl.multiple_of(c * TK, TK)
                s = _dot(k_s[g, pl.ds(r0, TK), :], qm_s[h])
                p = jnp.exp2(s - m)
                vt = vt_s[pl.ds(pl.multiple_of(h * DH, DH), DH), pl.ds(r0, TK)]
                return (l_acc + p.reshape(TK // 8, 8, TQ).sum(0), o_acc + _dot(vt, p.astype(BF16)))
            l_acc, o_acc = jax.lax.fori_loop(0, NC, acc, (jnp.zeros((8, TQ), F32), jnp.zeros((DH, TQ), F32)))
            finalize(h, l_acc, o_acc)
            lraw_s[...] = l_acc
            o_s[...] = o_acc
            return carry
        jax.lax.fori_loop(0, H, head, 0)
        for g in range(NG - 1):
            untranspose(g)
        carry_out(qk(H, 0, 0), qk(H, 0, 1), load_m(0, q_next))

    def attempt(state):
        a, _ = state

        @pl.when(a == 0)
        def _():
            jax.lax.fori_loop(0, NG, fast_body, 0)

        @pl.when(a == 1)
        def _():
            slow_attention()

        @pl.when(jnp.logical_or(step > 0, a > 0))
        def _():
            prev = jnp.where(a > 0, step, jnp.maximum(step - 1, 0))
            for r in range(NO):
                out_copy(r, prev).wait()

        finalize(H - 1, lraw_s[...], o_s[...])
        untranspose(NG - 1)
        l_all = l_s[...]
        ok = jnp.logical_and(l_all >= L_LO, l_all <= L_HI)
        n_bad = jnp.sum(jnp.where(ok, 0.0, 1.0))

        nf = TQ // FC
        h1 = {}
        ln2 = {}
        act = {}
        for r in range(nf):
            rows = slice(r * FC, (r + 1) * FC)
            attn = None
            for g in range(NG):
                part = _dot(on_s[g, rows, :], wo_v[128 * g:128 * (g + 1), :])
                attn = part if attn is None else attn + part
            h1[r] = x_v[pl.ds(pl.multiple_of(q0 + r * FC, FC), FC), :].astype(F32) + attn
            ln2[r] = _ln(h1[r]).astype(BF16)
        prep(nxt)
        for r in range(nf):
            gate = _dot_nt(ln2[r], w1_v[...])
            up = _dot_nt(ln2[r], w3_v[...])
            act[r] = (gate * jax.nn.sigmoid(gate) * up).astype(BF16)
        for r in range(nf):
            for u in range(FC // OC):
                y = _dot(act[r][u * OC:(u + 1) * OC], w2_v[...])
                k = r * (FC // OC) + u
                out_v[k * OC:(k + 1) * OC, :] = (h1[r][u * OC:(u + 1) * OC] + y).astype(BF16)
                out_copy(k, step).start()
        return a + 1, jnp.where(a == 0, (n_bad > 0.0).astype(jnp.int32), 0)

    jax.lax.while_loop(lambda s: s[0] < 1 + s[1], attempt, (jnp.int32(0), jnp.int32(0)))

    @pl.when(step == NQ - 1)
    def _():
        for r in range(NO):
            out_copy(r, step).wait()


@jax.jit
def pallas_sequential_preLN__softmax_full_mha__glu_gated_swiglu__prompt_kernel(
        A_x, A_wqkv, A_wo, B_x, B_w1, B_w3, B_w2):
    hbm = pl.BlockSpec(memory_space=pltpu.HBM)
    return pl.pallas_call(
        _kernel,
        grid=(NQ,),
        in_specs=[hbm] * 6,
        out_specs=hbm,
        out_shape=jax.ShapeDtypeStruct((1, S, D), BF16),
        scratch_shapes=[
            pltpu.VMEM((S, D), BF16),
            pltpu.VMEM((D, D), BF16),
            pltpu.VMEM((D, D), BF16),
            pltpu.VMEM((D, D), BF16),
            pltpu.VMEM((D, D), BF16),
            pltpu.VMEM((F, D), BF16),
            pltpu.VMEM((F, D), BF16),
            pltpu.VMEM((F, D), BF16),
            pltpu.VMEM((S, D), BF16),
            pltpu.VMEM((4, S, 128), BF16),
            pltpu.VMEM((D, S), BF16),
            pltpu.VMEM((D, S), BF16),
            pltpu.VMEM((H + 1, 128, TQ), BF16),
            pltpu.VMEM((D, TQ), BF16),
            pltpu.VMEM((NG, TQ, 128), BF16),
            pltpu.VMEM((H, 8, S), F32),
            pltpu.VMEM((H, TQ), F32),
            pltpu.VMEM((DH, TQ), F32),
            pltpu.VMEM((8, TQ), F32),
            pltpu.VMEM((TK, TQ), F32),
            pltpu.VMEM((TK, TQ), BF16),
            pltpu.VMEM((8, TQ), F32),
            pltpu.VMEM((TQ, D), BF16),
            pltpu.SMEM((HPB * NC,), jnp.int32),
            pltpu.SemaphoreType.DMA((NX + 7,)),
            pltpu.SemaphoreType.DMA((NO,)),
        ],
        compiler_params=pltpu.CompilerParams(
            dimension_semantics=("arbitrary",), vmem_limit_bytes=100 * 1024 * 1024),
        name="fused_block",
    )(A_x, A_wqkv, A_wo, B_w1.T, B_w3.T, B_w2)
```

```python
import math

import jax
import jax.numpy as jnp
import jax.experimental.pallas as pl
import jax.experimental.pallas.tpu as pltpu

S = 2048
D = 512
H = 32
DH = 16
F = 1376
TQ = 512
TK = 128
HPB = 8
DEPTH = 3
NQ = S // TQ
NC = S // TK
NG = H // HPB
RC = 512
NR = S // RC
XB = (0, 256, 512, 1024, 1536, 2048)
NX = len(XB) - 1
FC = 128
OC = 128
NO = TQ // OC
EPS = 1e-5
QSCALE = (DH ** -0.5) * math.log2(math.e)
L_LO = 2.0 ** -60
L_HI = 2.0 ** 64

QMAX = 959.0
KMAX = 1983.0
SHRINK = 1.0 - 2.0 ** -16

F32 = jnp.float32
BF16 = jnp.bfloat16
I8 = jnp.int8
I32 = jnp.int32
U32 = jnp.uint32


def _tree(op, xs):
    xs = list(xs)
    while len(xs) > 1:
        nxt = [op(xs[i], xs[i + 1]) for i in range(0, len(xs) - 1, 2)]
        if len(xs) % 2:
            nxt.append(xs[-1])
        xs = nxt
    return xs[0]


def _ln(x):
    m = jnp.mean(x, axis=-1, keepdims=True)
    xc = x - m
    v = jnp.mean(xc * xc, axis=-1, keepdims=True)
    return xc * jax.lax.rsqrt(v + EPS)


def _dot(a, b):
    return jnp.dot(a, b, preferred_element_type=F32)


def _dot_nt(a, b):
    return jax.lax.dot_general(a, b, (((1,), (1,)), ((), ())), preferred_element_type=F32)


MAGIC = 12582912.0


def _rnd(x):
    return (x + MAGIC) - MAGIC


def _round_to_i8_words(x):
    return pltpu.bitcast(pltpu.bitcast(x + MAGIC, I32).astype(I8), U32)


def _kernel(x_hbm, wqkv_hbm, wo_hbm, w1_hbm, w3_hbm, w2_hbm, out_hbm,
            x_v, wq_v, wk_v, wv_v, wo_v, w1_v, w3_v, w2_v,
            ln_s, k_s, kf_s, ki_s, vt_s, qt_s, qi_s, c_s, qm_s, ot_s, on_s, l_s, o_s, lraw_s, sc_s, pc_s, lc_s,
            rk_s, kc_s, out_v, zs, flag_s, sems, osems):
    step = pl.program_id(0)
    q0 = pl.multiple_of(step * TQ, TQ)
    q_next = pl.multiple_of(jnp.minimum(step + 1, NQ - 1) * TQ, TQ)

    def x_copy(c):
        n = XB[c + 1] - XB[c]
        return pltpu.make_async_copy(x_hbm.at[0, pl.ds(XB[c], n), :], x_v.at[pl.ds(XB[c], n), :], sems.at[c])

    def w_copy(i):
        src, dst = [(wqkv_hbm.at[:, pl.ds(D, D)], wk_v), (wqkv_hbm.at[:, pl.ds(2 * D, D)], wv_v),
                    (wqkv_hbm.at[:, pl.ds(0, D)], wq_v),
                    (wo_hbm, wo_v), (w1_hbm, w1_v), (w3_hbm, w3_v), (w2_hbm, w2_v)][i]
        return pltpu.make_async_copy(src, dst, sems.at[NX + i])

    def out_copy(r, tile):
        return pltpu.make_async_copy(out_v.at[pl.ds(r * OC, OC), :],
                                     out_hbm.at[0, pl.ds(pl.multiple_of(tile * TQ + r * OC, OC), OC), :],
                                     osems.at[r])

    def qk(h, pair, c, qoff, z=0):
        kk = pltpu.bitcast(ki_s[pair, c * (TK // 4):(c + 1) * (TK // 4), :], I8)
        qq = pltpu.bitcast(qi_s[h + z, :, pl.ds(qoff, TQ)], I8)
        return jnp.dot(kk, qq, preferred_element_type=I32)

    def softmax_num(s, cs):
        x = s.astype(F32).reshape(TK // 8, 8, TQ) * cs[None]
        p = jnp.exp2(x.reshape(TK, TQ))
        ll = _tree(jnp.add, [p[8 * i:8 * i + 8] for i in range(TK // 8)])
        return p.astype(BF16), ll

    def carry_out(ss, cs):
        pb, ll = softmax_num(ss[0], cs)
        pc_s[...] = pb
        lc_s[...] = ll
        for t in range(1, DEPTH):
            sc_s[t - 1] = ss[t]

    @pl.when(step == 0)
    def _prologue():
        for i in range(HPB * NC):
            zs[i] = 0
        x_copy(0).start()
        w_copy(0).start()
        for c in range(1, NX):
            x_copy(c).start()
        w_copy(1).start()
        w_copy(2).start()
        ot_s[...] = jnp.zeros(ot_s.shape, ot_s.dtype)
        o_s[...] = jnp.zeros(o_s.shape, F32)
        lraw_s[...] = jnp.ones(lraw_s.shape, F32)

        def ln_chunk(c):
            rows = slice(XB[c], XB[c + 1])
            ln_s[rows, :] = _ln(x_v[rows, :].astype(F32)).astype(BF16)

        def k_chunk(c):
            rows = slice(XB[c], XB[c + 1])
            k = _dot(ln_s[rows, :], wk_v[...])
            kf_s[rows, :] = k
            kb = k.astype(BF16)
            for g in range(4):
                k_s[g, rows, :] = kb[:, 128 * g:128 * (g + 1)]
            k3 = k.reshape(-1, 8, D)
            return jnp.max(jnp.abs(k3), axis=0), jnp.sum(k3 * k3, axis=0)

        x_copy(0).wait()
        ln_chunk(0)
        w_copy(0).wait()
        kabs = ksum = None
        for c in range(NX):
            if c + 1 < NX:
                x_copy(c + 1).wait()
            if c == NX - 2:
                w_copy(1).wait()
                w_copy(2).wait()
                for i in range(3, 7):
                    w_copy(i).start()
            ka, ks = k_chunk(c)
            kabs = ka if kabs is None else jnp.maximum(kabs, ka)
            ksum = ks if ksum is None else ksum + ks
            if c + 1 < NX:
                ln_chunk(c + 1)
            if c == NX - 2:
                wv_v[...] = wv_v[...].T
                wq_v[...] = wq_v[...].T
        vt_s[:, 0:RC] = _dot_nt(wv_v[...], ln_s[0:RC, :]).astype(BF16)
        kabs = jnp.max(kabs, axis=0, keepdims=True)
        ksum = jnp.sum(ksum, axis=0, keepdims=True)
        fine = kabs * kabs * float(S) <= 64.0 * ksum
        flag_s[0] = (jnp.sum(jnp.where(fine, 0.0, 1.0)) > 0.0).astype(I32)
        kabs = jnp.maximum(kabs, 1e-30)
        rk_s[...] = jnp.broadcast_to((KMAX * SHRINK) / kabs, (8, D))
        kc_s[...] = jnp.broadcast_to(kabs, (128, D)).T

        lane_blk = jax.lax.broadcasted_iota(I32, (1, 128), 1) // 16

        def project(c, carry):
            r0 = pl.multiple_of(c * RC, RC)
            ln = ln_s[pl.ds(r0, RC), :]
            q = _dot_nt(wq_v[...], ln) * QSCALE
            qt_s[:, pl.ds(r0, RC)] = q.astype(BF16)
            q = q * jnp.concatenate([kc_s[...]] * (RC // 128), axis=1)
            zero = jnp.zeros((16, RC), F32)
            for h in range(H):
                j = h % 8
                v = q[16 * h:16 * h + 16]
                a = jnp.maximum(jnp.abs(v[0:8]), jnp.abs(v[8:16]))
                for sh in (4, 2, 1):
                    a = jnp.maximum(a, pltpu.roll(a, sh, 0))
                a = jnp.maximum(a, 1e-30)
                r = pl.reciprocal(a, approx=True)
                inv = (r * (2.0 - a * r)) * (QMAX * SHRINK)
                t = _rnd((v.reshape(2, 8, RC) * inv[None]).reshape(16, RC))
                q1 = _rnd(t * (1.0 / 128.0))
                q0_ = t - 128.0 * q1
                grp = [16.0 * q1, q1, q0_, q0_ * 0.125]
                blocks = [zero] * 8
                for G in range(4):
                    blocks[(j + G) % 8] = grp[G]
                qi_s[h, :, pl.ds(r0, RC)] = _round_to_i8_words(jnp.concatenate(blocks, axis=0))
                c_s[h, :, pl.ds(r0, RC)] = a * (128.0 / (KMAX * QMAX * SHRINK * SHRINK))
            r1 = pl.multiple_of(jnp.minimum(c + 1, NR - 1) * RC, RC)
            vt_s[:, pl.ds(r1, RC)] = _dot_nt(wv_v[...], ln_s[pl.ds(r1, RC), :]).astype(BF16)
            rk = rk_s[0:1, :]
            KQ = 128
            for u in range(RC // KQ):
                t = _rnd(kf_s[pl.ds(r0 + u * KQ, KQ), :] * rk)
                k1 = _rnd(t * (1.0 / 128.0))
                k0 = t - 128.0 * k1
                limbs = [_round_to_i8_words(a) for a in (8.0 * k1, k0, k1, k0 * (1.0 / 16.0))]
                w0 = pl.multiple_of(c * (RC // 4) + u * (KQ // 4), KQ // 4)
                for g in range(4):
                    rolled = [limbs[G][:, 128 * g:128 * (g + 1)] for G in range(4)]
                    rolled = [rolled[0]] + [pltpu.roll(rolled[G], 16 * G, 1) for G in range(1, 4)]
                    for j in range(4):
                        sel = (lane_blk - j) % 4
                        ki_s[4 * g + j, pl.ds(w0, KQ // 4), :] = jnp.where(
                            sel == 0, rolled[0], jnp.where(sel == 1, rolled[1], jnp.where(sel == 2, rolled[2], rolled[3])))
            return carry

        jax.lax.fori_loop(0, NR, project, 0)
        carry_out([qk(0, 0, t, 0) for t in range(DEPTH)], c_s[0, :, 0:TQ])
        for i in range(3, 7):
            w_copy(i).wait()

    def pv(h, c, pb, ll, l_acc, o_acc):
        l_acc = ll if l_acc is None else l_acc + ll
        vt = vt_s[pl.ds(pl.multiple_of(h * DH, DH), DH), c * TK:(c + 1) * TK]
        oo = _dot(vt, pb)
        o_acc = oo if o_acc is None else o_acc + oo
        return l_acc, o_acc

    def load_c(h, qoff):
        return c_s[h, :, pl.ds(qoff, TQ)]

    def finalize(h, l_acc, o_acc, after=None):
        l = l_acc.sum(0, keepdims=True)
        if after is not None:
            z = on_s[after, 0:16, :].astype(F32)[0:1, :] * 0.0
            l = l + jnp.concatenate([z] * (TQ // 128), axis=1)
        l_s[pl.ds(h, 1), :] = l
        ot_s[pl.ds(pl.multiple_of(h * DH, DH), DH), :] = (o_acc * pl.reciprocal(l, approx=False)).astype(BF16)

    def untranspose(g):
        on_s[g] = ot_s[pl.ds(pl.multiple_of(g * 128, 128), 128), :].T

    def fast_body(i, carry):
        finalize(jnp.maximum(i * HPB - 1, 0), lraw_s[...], o_s[...])
        untranspose(jnp.maximum(i - 1, 0))
        items = [(i * HPB + j, (HPB // 2) * i + 4 * (j // 8) + j % 4, c, q0) for j in range(HPB) for c in range(NC)]
        last = i == NG - 1
        nh = jnp.where(last, 0, (i + 1) * HPB)
        npair = jnp.where(last, 0, (i + 1) * (HPB // 2))
        nq_ = pl.multiple_of(jnp.where(last, q_next, q0), TQ)
        items_all = items + [(nh, npair, c, nq_) for c in range(DEPTH)]
        ss = {t: sc_s[t - 1] for t in range(1, DEPTH)}
        cs = l_acc = o_acc = None
        for t, (h, _, c, _) in enumerate(items):
            ss[t + DEPTH] = qk(*items_all[t + DEPTH], z=zs[t])
            if c == 0:
                cs = load_c(h, q0)
                l_acc = o_acc = None
            if t == 0:
                pb, ll = pc_s[...], lc_s[...]
            else:
                pb, ll = softmax_num(ss.pop(t), cs)
            l_acc, o_acc = pv(h, c, pb, ll, l_acc, o_acc)
            if c == NC - 1:
                if t == len(items) - 1:
                    lraw_s[...] = l_acc
                    o_s[...] = o_acc
                else:
                    finalize(h, l_acc, o_acc, after=jnp.maximum(i - 1, 0) if t < NC else None)
        n = len(items)
        carry_out([ss[n + t] for t in range(DEPTH)], load_c(nh, nq_))
        return carry

    def slow_attention():
        def head(h, carry):
            g = h // 8
            qm_s[...] = jnp.zeros(qm_s.shape, BF16)
            qm_s[pl.ds(pl.multiple_of((h % 8) * DH, DH), DH), :] = qt_s[pl.ds(pl.multiple_of(h * DH, DH), DH), pl.ds(q0, TQ)]

            def mx(c, m_acc):
                r0 = pl.multiple_of(c * TK, TK)
                s = _dot(k_s[g, pl.ds(r0, TK), :], qm_s[...])
                return jnp.maximum(m_acc, jnp.max(s, axis=0, keepdims=True))
            m = jax.lax.fori_loop(0, NC, mx, jnp.full((1, TQ), -jnp.inf, F32))

            def acc(c, lo):
                l_acc, o_acc = lo
                r0 = pl.multiple_of(c * TK, TK)
                s = _dot(k_s[g, pl.ds(r0, TK), :], qm_s[...])
                p = jnp.exp2(s - m)
                vt = vt_s[pl.ds(pl.multiple_of(h * DH, DH), DH), pl.ds(r0, TK)]
                return (l_acc + p.reshape(TK // 8, 8, TQ).sum(0), o_acc + _dot(vt, p.astype(BF16)))
            l_acc, o_acc = jax.lax.fori_loop(0, NC, acc, (jnp.zeros((8, TQ), F32), jnp.zeros((DH, TQ), F32)))
            finalize(h, l_acc, o_acc)
            lraw_s[...] = l_acc
            o_s[...] = o_acc
            return carry
        jax.lax.fori_loop(0, H, head, 0)
        for g in range(NG - 1):
            untranspose(g)

    def attempt(state):
        a, _ = state

        @pl.when(a == 0)
        def _():
            jax.lax.fori_loop(0, NG, fast_body, 0)

        @pl.when(a == 1)
        def _():
            slow_attention()

        @pl.when(jnp.logical_or(step > 0, a > 0))
        def _():
            prev = jnp.where(a > 0, step, jnp.maximum(step - 1, 0))
            for r in range(NO):
                out_copy(r, prev).wait()

        finalize(H - 1, lraw_s[...], o_s[...])
        untranspose(NG - 1)
        l_all = l_s[...]
        ok = jnp.logical_and(l_all >= L_LO, l_all <= L_HI)
        n_bad = jnp.sum(jnp.where(ok, 0.0, 1.0))

        nf = TQ // FC
        h1 = {}
        ln2 = {}
        act = {}
        for r in range(nf):
            rows = slice(r * FC, (r + 1) * FC)
            attn = None
            for g in range(NG):
                part = _dot(on_s[g, rows, :], wo_v[128 * g:128 * (g + 1), :])
                attn = part if attn is None else attn + part
            h1[r] = x_v[pl.ds(pl.multiple_of(q0 + r * FC, FC), FC), :].astype(F32) + attn
            ln2[r] = _ln(h1[r]).astype(BF16)
        for r in range(nf):
            gate = _dot_nt(ln2[r], w1_v[...])
            up = _dot_nt(ln2[r], w3_v[...])
            act[r] = (gate * jax.nn.sigmoid(gate) * up).astype(BF16)
        for r in range(nf):
            for u in range(FC // OC):
                y = _dot(act[r][u * OC:(u + 1) * OC], w2_v[...])
                k = r * (FC // OC) + u
                out_v[k * OC:(k + 1) * OC, :] = (h1[r][u * OC:(u + 1) * OC] + y).astype(BF16)
                out_copy(k, step).start()
        redo = jnp.logical_or(n_bad > 0.0, flag_s[0] > 0)
        return a + 1, jnp.where(a == 0, redo.astype(jnp.int32), 0)

    jax.lax.while_loop(lambda s: s[0] < 1 + s[1], attempt, (jnp.int32(0), jnp.int32(0)))

    @pl.when(step == NQ - 1)
    def _():
        for r in range(NO):
            out_copy(r, step).wait()


@jax.jit
def pallas_sequential_preLN__softmax_full_mha__glu_gated_swiglu__prompt_kernel(
        A_x, A_wqkv, A_wo, B_x, B_w1, B_w3, B_w2):
    hbm = pl.BlockSpec(memory_space=pltpu.HBM)
    return pl.pallas_call(
        _kernel,
        grid=(NQ,),
        in_specs=[hbm] * 6,
        out_specs=hbm,
        out_shape=jax.ShapeDtypeStruct((1, S, D), BF16),
        scratch_shapes=[
            pltpu.VMEM((S, D), BF16),
            pltpu.VMEM((D, D), BF16),
            pltpu.VMEM((D, D), BF16),
            pltpu.VMEM((D, D), BF16),
            pltpu.VMEM((D, D), BF16),
            pltpu.VMEM((F, D), BF16),
            pltpu.VMEM((F, D), BF16),
            pltpu.VMEM((F, D), BF16),
            pltpu.VMEM((S, D), BF16),
            pltpu.VMEM((4, S, 128), BF16),
            pltpu.VMEM((S, D), F32),
            pltpu.VMEM((H // 2, S // 4, 128), U32),
            pltpu.VMEM((D, S), BF16),
            pltpu.VMEM((D, S), BF16),
            pltpu.VMEM((H, 32, S), U32),
            pltpu.VMEM((H, 8, S), F32),
            pltpu.VMEM((128, TQ), BF16),
            pltpu.VMEM((D, TQ), BF16),
            pltpu.VMEM((4, TQ, 128), BF16),
            pltpu.VMEM((H, TQ), F32),
            pltpu.VMEM((DH, TQ), F32),
            pltpu.VMEM((8, TQ), F32),
            pltpu.VMEM((DEPTH - 1, TK, TQ), I32),
            pltpu.VMEM((TK, TQ), BF16),
            pltpu.VMEM((8, TQ), F32),
            pltpu.VMEM((8, D), F32),
            pltpu.VMEM((D, 128), F32),
            pltpu.VMEM((TQ, D), BF16),
            pltpu.SMEM((HPB * NC,), jnp.int32),
            pltpu.SMEM((1,), jnp.int32),
            pltpu.SemaphoreType.DMA((NX + 7,)),
            pltpu.SemaphoreType.DMA((NO,)),
        ],
        compiler_params=pltpu.CompilerParams(
            dimension_semantics=("arbitrary",), vmem_limit_bytes=100 * 1024 * 1024),
        name="fused_block",
    )(A_x, A_wqkv, A_wo, B_w1.T, B_w3.T, B_w2)
```

```python
import math

import jax
import jax.numpy as jnp
import jax.experimental.pallas as pl
import jax.experimental.pallas.tpu as pltpu

S = 2048
D = 512
H = 32
DH = 16
F = 1376
TQ = 512
TK = 128
HPB = 16
GPB = HPB // 8
DEPTH = 3
NQ = S // TQ
NC = S // TK
NG = H // HPB
RC = 512
NR = S // RC
XB = (0, 256, 512, 1024, 1536, 2048)
NX = len(XB) - 1
FC = 128
OC = 128
NO = TQ // OC
EPS = 1e-5
QSCALE = (DH ** -0.5) * math.log2(math.e)
L_LO = 2.0 ** -60
L_HI = 2.0 ** 64

QMAX = 959.0
KMAX = 1983.0
SHRINK = 1.0 - 2.0 ** -16

F32 = jnp.float32
BF16 = jnp.bfloat16
I8 = jnp.int8
I32 = jnp.int32
U32 = jnp.uint32


def _tree(op, xs):
    xs = list(xs)
    while len(xs) > 1:
        nxt = [op(xs[i], xs[i + 1]) for i in range(0, len(xs) - 1, 2)]
        if len(xs) % 2:
            nxt.append(xs[-1])
        xs = nxt
    return xs[0]


def _ln(x):
    m = jnp.mean(x, axis=-1, keepdims=True)
    xc = x - m
    v = jnp.mean(xc * xc, axis=-1, keepdims=True)
    return xc * jax.lax.rsqrt(v + EPS)


def _dot(a, b):
    return jnp.dot(a, b, preferred_element_type=F32)


def _dot_nt(a, b):
    return jax.lax.dot_general(a, b, (((1,), (1,)), ((), ())), preferred_element_type=F32)


MAGIC = 12582912.0


def _rnd(x):
    return (x + MAGIC) - MAGIC


def _round_to_i8_words(x):
    return pltpu.bitcast(pltpu.bitcast(x + MAGIC, I32).astype(I8), U32)


def _kernel(x_hbm, wqkv_hbm, wo_hbm, w1_hbm, w3_hbm, w2_hbm, out_hbm,
            x_v, wq_v, wk_v, wv_v, wo_v, w1_v, w3_v, w2_v,
            ln_s, k_s, kf_s, ki_s, vt_s, qt_s, qi_s, c_s, qm_s, ot_s, on_s, l_s, o_s, lraw_s, sc_s, pc_s, lc_s,
            rk_s, kc_s, out_v, zs, flag_s, sems, osems):
    step = pl.program_id(0)
    q0 = pl.multiple_of(step * TQ, TQ)
    q_next = pl.multiple_of(jnp.minimum(step + 1, NQ - 1) * TQ, TQ)

    def x_copy(c):
        n = XB[c + 1] - XB[c]
        return pltpu.make_async_copy(x_hbm.at[0, pl.ds(XB[c], n), :], x_v.at[pl.ds(XB[c], n), :], sems.at[c])

    def w_copy(i):
        src, dst = [(wqkv_hbm.at[:, pl.ds(D, D)], wk_v), (wqkv_hbm.at[:, pl.ds(2 * D, D)], wv_v),
                    (wqkv_hbm.at[:, pl.ds(0, D)], wq_v),
                    (wo_hbm, wo_v), (w1_hbm, w1_v), (w3_hbm, w3_v), (w2_hbm, w2_v)][i]
        return pltpu.make_async_copy(src, dst, sems.at[NX + i])

    def out_copy(r, tile):
        return pltpu.make_async_copy(out_v.at[pl.ds(r * OC, OC), :],
                                     out_hbm.at[0, pl.ds(pl.multiple_of(tile * TQ + r * OC, OC), OC), :],
                                     osems.at[r])

    def qk(h, pair, c, qoff, z=0):
        kk = pltpu.bitcast(ki_s[pair, c * (TK // 4):(c + 1) * (TK // 4), :], I8)
        qq = pltpu.bitcast(qi_s[h + z, :, pl.ds(qoff, TQ)], I8)
        return jnp.dot(kk, qq, preferred_element_type=I32)

    def softmax_num(s, cs):
        x = s.astype(F32).reshape(TK // 8, 8, TQ) * cs[None]
        p = jnp.exp2(x.reshape(TK, TQ))
        ll = _tree(jnp.add, [p[8 * i:8 * i + 8] for i in range(TK // 8)])
        return p.astype(BF16), ll

    def carry_out(ss, cs):
        pb, ll = softmax_num(ss[0], cs)
        pc_s[...] = pb
        lc_s[...] = ll
        for t in range(1, DEPTH):
            sc_s[t - 1] = ss[t]

    @pl.when(step == 0)
    def _prologue():
        for i in range(HPB * NC):
            zs[i] = 0
        x_copy(0).start()
        w_copy(0).start()
        for c in range(1, NX):
            x_copy(c).start()
        w_copy(1).start()
        w_copy(2).start()
        ot_s[...] = jnp.zeros(ot_s.shape, ot_s.dtype)
        o_s[...] = jnp.zeros(o_s.shape, F32)
        lraw_s[...] = jnp.ones(lraw_s.shape, F32)

        def ln_chunk(c):
            rows = slice(XB[c], XB[c + 1])
            ln_s[rows, :] = _ln(x_v[rows, :].astype(F32)).astype(BF16)

        def k_chunk(c):
            rows = slice(XB[c], XB[c + 1])
            k = _dot(ln_s[rows, :], wk_v[...])
            kf_s[rows, :] = k
            kb = k.astype(BF16)
            for g in range(4):
                k_s[g, rows, :] = kb[:, 128 * g:128 * (g + 1)]
            k3 = k.reshape(-1, 8, D)
            return jnp.max(jnp.abs(k3), axis=0), jnp.sum(k3 * k3, axis=0)

        x_copy(0).wait()
        ln_chunk(0)
        w_copy(0).wait()
        kabs = ksum = None
        for c in range(NX):
            if c + 1 < NX:
                x_copy(c + 1).wait()
            if c == NX - 2:
                w_copy(1).wait()
                w_copy(2).wait()
                for i in range(3, 7):
                    w_copy(i).start()
            ka, ks = k_chunk(c)
            kabs = ka if kabs is None else jnp.maximum(kabs, ka)
            ksum = ks if ksum is None else ksum + ks
            if c + 1 < NX:
                ln_chunk(c + 1)
            if c == NX - 2:
                wv_v[...] = wv_v[...].T
                wq_v[...] = wq_v[...].T
        vt_s[:, 0:RC] = _dot_nt(wv_v[...], ln_s[0:RC, :]).astype(BF16)
        kabs = jnp.max(kabs, axis=0, keepdims=True)
        ksum = jnp.sum(ksum, axis=0, keepdims=True)
        fine = kabs * kabs * float(S) <= 64.0 * ksum
        flag_s[0] = (jnp.sum(jnp.where(fine, 0.0, 1.0)) > 0.0).astype(I32)
        kabs = jnp.maximum(kabs, 1e-30)
        rk_s[...] = jnp.broadcast_to((KMAX * SHRINK) / kabs, (8, D))
        kc_s[...] = jnp.broadcast_to(kabs, (128, D)).T

        lane_blk = jax.lax.broadcasted_iota(I32, (1, 128), 1) // 16

        def project(c, carry):
            r0 = pl.multiple_of(c * RC, RC)
            ln = ln_s[pl.ds(r0, RC), :]
            q = _dot_nt(wq_v[...], ln) * QSCALE
            qt_s[:, pl.ds(r0, RC)] = q.astype(BF16)
            q = q * jnp.concatenate([kc_s[...]] * (RC // 128), axis=1)
            zero = jnp.zeros((16, RC), F32)
            for h in range(H):
                j = h % 8
                v = q[16 * h:16 * h + 16]
                a = jnp.maximum(jnp.abs(v[0:8]), jnp.abs(v[8:16]))
                for sh in (4, 2, 1):
                    a = jnp.maximum(a, pltpu.roll(a, sh, 0))
                a = jnp.maximum(a, 1e-30)
                r = pl.reciprocal(a, approx=True)
                inv = (r * (2.0 - a * r)) * (QMAX * SHRINK)
                t = _rnd((v.reshape(2, 8, RC) * inv[None]).reshape(16, RC))
                q1 = _rnd(t * (1.0 / 128.0))
                q0_ = t - 128.0 * q1
                grp = [16.0 * q1, q1, q0_, q0_ * 0.125]
                blocks = [zero] * 8
                for G in range(4):
                    blocks[(j + G) % 8] = grp[G]
                qi_s[h, :, pl.ds(r0, RC)] = _round_to_i8_words(jnp.concatenate(blocks, axis=0))
                c_s[h, :, pl.ds(r0, RC)] = a * (128.0 / (KMAX * QMAX * SHRINK * SHRINK))
            r1 = pl.multiple_of(jnp.minimum(c + 1, NR - 1) * RC, RC)
            vt_s[:, pl.ds(r1, RC)] = _dot_nt(wv_v[...], ln_s[pl.ds(r1, RC), :]).astype(BF16)
            rk = rk_s[0:1, :]
            KQ = 128
            for u in range(RC // KQ):
                t = _rnd(kf_s[pl.ds(r0 + u * KQ, KQ), :] * rk)
                k1 = _rnd(t * (1.0 / 128.0))
                k0 = t - 128.0 * k1
                limbs = [_round_to_i8_words(a) for a in (8.0 * k1, k0, k1, k0 * (1.0 / 16.0))]
                w0 = pl.multiple_of(c * (RC // 4) + u * (KQ // 4), KQ // 4)
                for g in range(4):
                    rolled = [limbs[G][:, 128 * g:128 * (g + 1)] for G in range(4)]
                    rolled = [rolled[0]] + [pltpu.roll(rolled[G], 16 * G, 1) for G in range(1, 4)]
                    for j in range(4):
                        sel = (lane_blk - j) % 4
                        ki_s[4 * g + j, pl.ds(w0, KQ // 4), :] = jnp.where(
                            sel == 0, rolled[0], jnp.where(sel == 1, rolled[1], jnp.where(sel == 2, rolled[2], rolled[3])))
            return carry

        jax.lax.fori_loop(0, NR, project, 0)
        carry_out([qk(0, 0, t, 0) for t in range(DEPTH)], c_s[0, :, 0:TQ])
        for i in range(3, 7):
            w_copy(i).wait()

    def pv(h, c, pb, ll, l_acc, o_acc):
        l_acc = ll if l_acc is None else l_acc + ll
        vt = vt_s[pl.ds(pl.multiple_of(h * DH, DH), DH), c * TK:(c + 1) * TK]
        oo = _dot(vt, pb)
        o_acc = oo if o_acc is None else o_acc + oo
        return l_acc, o_acc

    def load_c(h, qoff):
        return c_s[h, :, pl.ds(qoff, TQ)]

    def finalize(h, l_acc, o_acc, after=None):
        l = l_acc.sum(0, keepdims=True)
        if after is not None:
            z = on_s[after, 0:16, :].astype(F32)[0:1, :] * 0.0
            l = l + jnp.concatenate([z] * (TQ // 128), axis=1)
        l_s[pl.ds(h, 1), :] = l
        ot_s[pl.ds(pl.multiple_of(h * DH, DH), DH), :] = (o_acc * pl.reciprocal(l, approx=False)).astype(BF16)

    def untranspose(g):
        on_s[g] = ot_s[pl.ds(pl.multiple_of(g * 128, 128), 128), :].T

    def fast_body(i, carry):
        finalize(jnp.maximum(i * HPB - 1, 0), lraw_s[...], o_s[...])
        untranspose(jnp.maximum(i * GPB - 1, 0))
        items = [(i * HPB + j, (HPB // 2) * i + 4 * (j // 8) + j % 4, c, q0) for j in range(HPB) for c in range(NC)]
        last = i == NG - 1
        nh = jnp.where(last, 0, (i + 1) * HPB)
        npair = jnp.where(last, 0, (i + 1) * (HPB // 2))
        nq_ = pl.multiple_of(jnp.where(last, q_next, q0), TQ)
        items_all = items + [(nh, npair, c, nq_) for c in range(DEPTH)]
        ss = {t: sc_s[t - 1] for t in range(1, DEPTH)}
        cs = l_acc = o_acc = None
        for t, (h, _, c, _) in enumerate(items):
            ss[t + DEPTH] = qk(*items_all[t + DEPTH], z=zs[t])
            if c == 0:
                cs = load_c(h, q0)
                l_acc = o_acc = None
            if t == 0:
                pb, ll = pc_s[...], lc_s[...]
            else:
                pb, ll = softmax_num(ss.pop(t), cs)
            l_acc, o_acc = pv(h, c, pb, ll, l_acc, o_acc)
            if c == NC - 1:
                if t == len(items) - 1:
                    lraw_s[...] = l_acc
                    o_s[...] = o_acc
                else:
                    j = t // NC
                    finalize(h, l_acc, o_acc, after=jnp.maximum(i * GPB + j // 8 - 1, 0) if j % 8 == 0 else None)
                    if j % 8 == 7:
                        untranspose(i * GPB + j // 8)
        n = len(items)
        carry_out([ss[n + t] for t in range(DEPTH)], load_c(nh, nq_))
        return carry

    def slow_attention():
        def head(h, carry):
            g = h // 8
            qm_s[...] = jnp.zeros(qm_s.shape, BF16)
            qm_s[pl.ds(pl.multiple_of((h % 8) * DH, DH), DH), :] = qt_s[pl.ds(pl.multiple_of(h * DH, DH), DH), pl.ds(q0, TQ)]

            def mx(c, m_acc):
                r0 = pl.multiple_of(c * TK, TK)
                s = _dot(k_s[g, pl.ds(r0, TK), :], qm_s[...])
                return jnp.maximum(m_acc, jnp.max(s, axis=0, keepdims=True))
            m = jax.lax.fori_loop(0, NC, mx, jnp.full((1, TQ), -jnp.inf, F32))

            def acc(c, lo):
                l_acc, o_acc = lo
                r0 = pl.multiple_of(c * TK, TK)
                s = _dot(k_s[g, pl.ds(r0, TK), :], qm_s[...])
                p = jnp.exp2(s - m)
                vt = vt_s[pl.ds(pl.multiple_of(h * DH, DH), DH), pl.ds(r0, TK)]
                return (l_acc + p.reshape(TK // 8, 8, TQ).sum(0), o_acc + _dot(vt, p.astype(BF16)))
            l_acc, o_acc = jax.lax.fori_loop(0, NC, acc, (jnp.zeros((8, TQ), F32), jnp.zeros((DH, TQ), F32)))
            finalize(h, l_acc, o_acc)
            lraw_s[...] = l_acc
            o_s[...] = o_acc
            return carry
        jax.lax.fori_loop(0, H, head, 0)
        for g in range(3):
            untranspose(g)

    def attempt(state):
        a, _ = state

        @pl.when(a == 0)
        def _():
            jax.lax.fori_loop(0, NG, fast_body, 0)

        @pl.when(a == 1)
        def _():
            slow_attention()

        @pl.when(jnp.logical_or(step > 0, a > 0))
        def _():
            prev = jnp.where(a > 0, step, jnp.maximum(step - 1, 0))
            for r in range(NO):
                out_copy(r, prev).wait()

        finalize(H - 1, lraw_s[...], o_s[...])
        untranspose(3)
        l_all = l_s[...]
        ok = jnp.logical_and(l_all >= L_LO, l_all <= L_HI)
        n_bad = jnp.sum(jnp.where(ok, 0.0, 1.0))

        nf = TQ // FC
        h1 = {}
        ln2 = {}
        act = {}
        for r in range(nf):
            rows = slice(r * FC, (r + 1) * FC)
            attn = None
            for g in range(4):
                part = _dot(on_s[g, rows, :], wo_v[128 * g:128 * (g + 1), :])
                attn = part if attn is None else attn + part
            h1[r] = x_v[pl.ds(pl.multiple_of(q0 + r * FC, FC), FC), :].astype(F32) + attn
            ln2[r] = _ln(h1[r]).astype(BF16)
        for r in range(nf):
            gate = _dot_nt(ln2[r], w1_v[...])
            up = _dot_nt(ln2[r], w3_v[...])
            act[r] = (gate * jax.nn.sigmoid(gate) * up).astype(BF16)
        for r in range(nf):
            for u in range(FC // OC):
                y = _dot(act[r][u * OC:(u + 1) * OC], w2_v[...])
                k = r * (FC // OC) + u
                out_v[k * OC:(k + 1) * OC, :] = (h1[r][u * OC:(u + 1) * OC] + y).astype(BF16)
                out_copy(k, step).start()
        redo = jnp.logical_or(n_bad > 0.0, flag_s[0] > 0)
        return a + 1, jnp.where(a == 0, redo.astype(jnp.int32), 0)

    jax.lax.while_loop(lambda s: s[0] < 1 + s[1], attempt, (jnp.int32(0), jnp.int32(0)))

    @pl.when(step == NQ - 1)
    def _():
        for r in range(NO):
            out_copy(r, step).wait()


@jax.jit
def pallas_sequential_preLN__softmax_full_mha__glu_gated_swiglu__prompt_kernel(
        A_x, A_wqkv, A_wo, B_x, B_w1, B_w3, B_w2):
    hbm = pl.BlockSpec(memory_space=pltpu.HBM)
    return pl.pallas_call(
        _kernel,
        grid=(NQ,),
        in_specs=[hbm] * 6,
        out_specs=hbm,
        out_shape=jax.ShapeDtypeStruct((1, S, D), BF16),
        scratch_shapes=[
            pltpu.VMEM((S, D), BF16),
            pltpu.VMEM((D, D), BF16),
            pltpu.VMEM((D, D), BF16),
            pltpu.VMEM((D, D), BF16),
            pltpu.VMEM((D, D), BF16),
            pltpu.VMEM((F, D), BF16),
            pltpu.VMEM((F, D), BF16),
            pltpu.VMEM((F, D), BF16),
            pltpu.VMEM((S, D), BF16),
            pltpu.VMEM((4, S, 128), BF16),
            pltpu.VMEM((S, D), F32),
            pltpu.VMEM((H // 2, S // 4, 128), U32),
            pltpu.VMEM((D, S), BF16),
            pltpu.VMEM((D, S), BF16),
            pltpu.VMEM((H, 32, S), U32),
            pltpu.VMEM((H, 8, S), F32),
            pltpu.VMEM((128, TQ), BF16),
            pltpu.VMEM((D, TQ), BF16),
            pltpu.VMEM((4, TQ, 128), BF16),
            pltpu.VMEM((H, TQ), F32),
            pltpu.VMEM((DH, TQ), F32),
            pltpu.VMEM((8, TQ), F32),
            pltpu.VMEM((DEPTH - 1, TK, TQ), I32),
            pltpu.VMEM((TK, TQ), BF16),
            pltpu.VMEM((8, TQ), F32),
            pltpu.VMEM((8, D), F32),
            pltpu.VMEM((D, 128), F32),
            pltpu.VMEM((TQ, D), BF16),
            pltpu.SMEM((HPB * NC,), jnp.int32),
            pltpu.SMEM((1,), jnp.int32),
            pltpu.SemaphoreType.DMA((NX + 7,)),
            pltpu.SemaphoreType.DMA((NO,)),
        ],
        compiler_params=pltpu.CompilerParams(
            dimension_semantics=("arbitrary",), vmem_limit_bytes=100 * 1024 * 1024),
        name="fused_block",
    )(A_x, A_wqkv, A_wo, B_w1.T, B_w3.T, B_w2)
```

```python
import math

import jax
import jax.numpy as jnp
import jax.experimental.pallas as pl
import jax.experimental.pallas.tpu as pltpu

S = 2048
D = 512
H = 32
DH = 16
F = 1376
TQ = 512
TK = 128
HPB = 16
GPB = HPB // 8
GRP = 2
DEPTH = 2
NQ = S // TQ
NC = S // TK
NG = H // HPB
RC = 512
NR = S // RC
XB = (0, 256, 512, 1024, 1536, 2048)
NX = len(XB) - 1
FC = 128
OC = 128
NO = TQ // OC
EPS = 1e-5
QSCALE = (DH ** -0.5) * math.log2(math.e)
L_LO = 2.0 ** -60
L_HI = 2.0 ** 64

QMAX = 959.0
KMAX = 1983.0
SHRINK = 1.0 - 2.0 ** -16

F32 = jnp.float32
BF16 = jnp.bfloat16
I8 = jnp.int8
I32 = jnp.int32
U32 = jnp.uint32


def _tree(op, xs):
    xs = list(xs)
    while len(xs) > 1:
        nxt = [op(xs[i], xs[i + 1]) for i in range(0, len(xs) - 1, 2)]
        if len(xs) % 2:
            nxt.append(xs[-1])
        xs = nxt
    return xs[0]


def _ln(x):
    m = jnp.mean(x, axis=-1, keepdims=True)
    xc = x - m
    v = jnp.mean(xc * xc, axis=-1, keepdims=True)
    return xc * jax.lax.rsqrt(v + EPS)


def _dot(a, b):
    return jnp.dot(a, b, preferred_element_type=F32)


def _dot_nt(a, b):
    return jax.lax.dot_general(a, b, (((1,), (1,)), ((), ())), preferred_element_type=F32)


MAGIC = 12582912.0


def _rnd(x):
    return (x + MAGIC) - MAGIC


def _round_to_i8_words(x):
    return pltpu.bitcast(pltpu.bitcast(x + MAGIC, I32).astype(I8), U32)


def _kernel(x_hbm, wqkv_hbm, wo_hbm, w1_hbm, w3_hbm, w2_hbm, out_hbm,
            x_v, wq_v, wk_v, wv_v, wo_v, w1_v, w3_v, w2_v,
            ln_s, k_s, kf_s, ki_s, vt_s, qt_s, qi_s, c_s, qm_s, ot_s, on_s, l_s, o_s, lraw_s, sc_s, pc_s, lc_s,
            rk_s, kc_s, out_v, zs, flag_s, sems, osems):
    step = pl.program_id(0)
    q0 = pl.multiple_of(step * TQ, TQ)
    q_next = pl.multiple_of(jnp.minimum(step + 1, NQ - 1) * TQ, TQ)

    def x_copy(c):
        n = XB[c + 1] - XB[c]
        return pltpu.make_async_copy(x_hbm.at[0, pl.ds(XB[c], n), :], x_v.at[pl.ds(XB[c], n), :], sems.at[c])

    def w_copy(i):
        src, dst = [(wqkv_hbm.at[:, pl.ds(D, D)], wk_v), (wqkv_hbm.at[:, pl.ds(2 * D, D)], wv_v),
                    (wqkv_hbm.at[:, pl.ds(0, D)], wq_v),
                    (wo_hbm, wo_v), (w1_hbm, w1_v), (w3_hbm, w3_v), (w2_hbm, w2_v)][i]
        return pltpu.make_async_copy(src, dst, sems.at[NX + i])

    def out_copy(r, tile):
        return pltpu.make_async_copy(out_v.at[pl.ds(r * OC, OC), :],
                                     out_hbm.at[0, pl.ds(pl.multiple_of(tile * TQ + r * OC, OC), OC), :],
                                     osems.at[r])

    def qk(h, pair, c, qoff, z=0, n=1):
        kk = pltpu.bitcast(ki_s[pair, c * (TK // 4):(c + n) * (TK // 4), :], I8)
        qq = pltpu.bitcast(qi_s[h + z, :, pl.ds(qoff, TQ)], I8)
        return jnp.dot(kk, qq, preferred_element_type=I32)

    def softmax_num(s, cs):
        x = s.astype(F32).reshape(TK // 8, 8, TQ) * cs[None]
        p = jnp.exp2(x.reshape(TK, TQ))
        ll = _tree(jnp.add, [p[8 * i:8 * i + 8] for i in range(TK // 8)])
        return p.astype(BF16), ll

    def carry_out(ss, cs):
        pb, ll = softmax_num(ss[0], cs)
        pc_s[...] = pb
        lc_s[...] = ll
        for t in range(1, DEPTH):
            sc_s[t - 1] = ss[t]

    @pl.when(step == 0)
    def _prologue():
        for i in range(HPB * NC):
            zs[i] = 0
        x_copy(0).start()
        w_copy(0).start()
        for c in range(1, NX):
            x_copy(c).start()
        w_copy(1).start()
        w_copy(2).start()
        ot_s[...] = jnp.zeros(ot_s.shape, ot_s.dtype)
        o_s[...] = jnp.zeros(o_s.shape, F32)
        lraw_s[...] = jnp.ones(lraw_s.shape, F32)

        def ln_chunk(c):
            rows = slice(XB[c], XB[c + 1])
            ln_s[rows, :] = _ln(x_v[rows, :].astype(F32)).astype(BF16)

        def k_chunk(c):
            rows = slice(XB[c], XB[c + 1])
            k = _dot(ln_s[rows, :], wk_v[...])
            kf_s[rows, :] = k
            kb = k.astype(BF16)
            for g in range(4):
                k_s[g, rows, :] = kb[:, 128 * g:128 * (g + 1)]
            k3 = k.reshape(-1, 8, D)
            return jnp.max(jnp.abs(k3), axis=0), jnp.sum(k3 * k3, axis=0)

        x_copy(0).wait()
        ln_chunk(0)
        w_copy(0).wait()
        kabs = ksum = None
        for c in range(NX):
            if c + 1 < NX:
                x_copy(c + 1).wait()
            if c == NX - 2:
                w_copy(1).wait()
                w_copy(2).wait()
                for i in range(3, 7):
                    w_copy(i).start()
            ka, ks = k_chunk(c)
            kabs = ka if kabs is None else jnp.maximum(kabs, ka)
            ksum = ks if ksum is None else ksum + ks
            if c + 1 < NX:
                ln_chunk(c + 1)
            if c == NX - 2:
                wv_v[...] = wv_v[...].T
                wq_v[...] = wq_v[...].T
        vt_s[:, 0:RC] = _dot_nt(wv_v[...], ln_s[0:RC, :]).astype(BF16)
        kabs = jnp.max(kabs, axis=0, keepdims=True)
        ksum = jnp.sum(ksum, axis=0, keepdims=True)
        fine = kabs * kabs * float(S) <= 64.0 * ksum
        flag_s[0] = (jnp.sum(jnp.where(fine, 0.0, 1.0)) > 0.0).astype(I32)
        kabs = jnp.maximum(kabs, 1e-30)
        rk_s[...] = jnp.broadcast_to((KMAX * SHRINK) / kabs, (8, D))
        kc_s[...] = jnp.broadcast_to(kabs, (128, D)).T

        lane_blk = jax.lax.broadcasted_iota(I32, (1, 128), 1) // 16

        def project(c, carry):
            r0 = pl.multiple_of(c * RC, RC)
            ln = ln_s[pl.ds(r0, RC), :]
            q = _dot_nt(wq_v[...], ln) * QSCALE
            qt_s[:, pl.ds(r0, RC)] = q.astype(BF16)
            q = q * jnp.concatenate([kc_s[...]] * (RC // 128), axis=1)
            zero = jnp.zeros((16, RC), F32)
            for h in range(H):
                j = h % 8
                v = q[16 * h:16 * h + 16]
                a = jnp.maximum(jnp.abs(v[0:8]), jnp.abs(v[8:16]))
                for sh in (4, 2, 1):
                    a = jnp.maximum(a, pltpu.roll(a, sh, 0))
                a = jnp.maximum(a, 1e-30)
                r = pl.reciprocal(a, approx=True)
                inv = (r * (2.0 - a * r)) * (QMAX * SHRINK)
                t = _rnd((v.reshape(2, 8, RC) * inv[None]).reshape(16, RC))
                q1 = _rnd(t * (1.0 / 128.0))
                q0_ = t - 128.0 * q1
                grp = [16.0 * q1, q1, q0_, q0_ * 0.125]
                blocks = [zero] * 8
                for G in range(4):
                    blocks[(j + G) % 8] = grp[G]
                qi_s[h, :, pl.ds(r0, RC)] = _round_to_i8_words(jnp.concatenate(blocks, axis=0))
                c_s[h, :, pl.ds(r0, RC)] = a * (128.0 / (KMAX * QMAX * SHRINK * SHRINK))
            r1 = pl.multiple_of(jnp.minimum(c + 1, NR - 1) * RC, RC)
            vt_s[:, pl.ds(r1, RC)] = _dot_nt(wv_v[...], ln_s[pl.ds(r1, RC), :]).astype(BF16)
            rk = rk_s[0:1, :]
            KQ = 128
            for u in range(RC // KQ):
                t = _rnd(kf_s[pl.ds(r0 + u * KQ, KQ), :] * rk)
                k1 = _rnd(t * (1.0 / 128.0))
                k0 = t - 128.0 * k1
                limbs = [_round_to_i8_words(a) for a in (8.0 * k1, k0, k1, k0 * (1.0 / 16.0))]
                w0 = pl.multiple_of(c * (RC // 4) + u * (KQ // 4), KQ // 4)
                for g in range(4):
                    rolled = [limbs[G][:, 128 * g:128 * (g + 1)] for G in range(4)]
                    rolled = [rolled[0]] + [pltpu.roll(rolled[G], 16 * G, 1) for G in range(1, 4)]
                    for j in range(4):
                        sel = (lane_blk - j) % 4
                        ki_s[4 * g + j, pl.ds(w0, KQ // 4), :] = jnp.where(
                            sel == 0, rolled[0], jnp.where(sel == 1, rolled[1], jnp.where(sel == 2, rolled[2], rolled[3])))
            return carry

        jax.lax.fori_loop(0, NR, project, 0)
        carry_out([qk(0, 0, t, 0) for t in range(DEPTH)], c_s[0, :, 0:TQ])
        for i in range(3, 7):
            w_copy(i).wait()

    def pv(h, c, pb, ll, l_acc, o_acc):
        l_acc = ll if l_acc is None else l_acc + ll
        vt = vt_s[pl.ds(pl.multiple_of(h * DH, DH), DH), c * TK:(c + 1) * TK]
        oo = _dot(vt, pb)
        o_acc = oo if o_acc is None else o_acc + oo
        return l_acc, o_acc

    def load_c(h, qoff):
        return c_s[h, :, pl.ds(qoff, TQ)]

    def finalize(h, l_acc, o_acc, after=None):
        l = l_acc.sum(0, keepdims=True)
        if after is not None:
            z = on_s[after, 0:16, :].astype(F32)[0:1, :] * 0.0
            l = l + jnp.concatenate([z] * (TQ // 128), axis=1)
        l_s[pl.ds(h, 1), :] = l
        ot_s[pl.ds(pl.multiple_of(h * DH, DH), DH), :] = (o_acc * pl.reciprocal(l, approx=False)).astype(BF16)

    def untranspose(g):
        on_s[g] = ot_s[pl.ds(pl.multiple_of(g * 128, 128), 128), :].T

    def fast_body(i, carry):
        finalize(jnp.maximum(i * HPB - 1, 0), lraw_s[...], o_s[...])
        untranspose(jnp.maximum(i * GPB - 1, 0))
        items = [(i * HPB + j, (HPB // 2) * i + 4 * (j // 8) + j % 4, c, q0) for j in range(HPB) for c in range(NC)]
        last = i == NG - 1
        nh = jnp.where(last, 0, (i + 1) * HPB)
        npair = jnp.where(last, 0, (i + 1) * (HPB // 2))
        nq_ = pl.multiple_of(jnp.where(last, q_next, q0), TQ)
        items_all = items + [(nh, npair, c, nq_) for c in range(DEPTH)]
        ss = {t: sc_s[t - 1] for t in range(1, DEPTH)}
        cs = l_acc = o_acc = None
        issued = DEPTH
        for t, (h, _, c, _) in enumerate(items):
            if t % GRP == 0:
                s2 = qk(*items_all[issued], z=zs[issued - DEPTH], n=GRP)
                ss[issued] = s2[0:TK]
                ss[issued + 1] = s2[TK:2 * TK]
                issued += 2
            if c == 0:
                cs = load_c(h, q0)
                l_acc = o_acc = None
            if t == 0:
                pb, ll = pc_s[...], lc_s[...]
            else:
                pb, ll = softmax_num(ss.pop(t), cs)
            l_acc, o_acc = pv(h, c, pb, ll, l_acc, o_acc)
            if c == NC - 1:
                if t == len(items) - 1:
                    lraw_s[...] = l_acc
                    o_s[...] = o_acc
                else:
                    j = t // NC
                    finalize(h, l_acc, o_acc, after=jnp.maximum(i * GPB + j // 8 - 1, 0) if j % 8 == 0 else None)
                    if j % 8 == 7:
                        untranspose(i * GPB + j // 8)
        n = len(items)
        carry_out([ss[n + t] for t in range(DEPTH)], load_c(nh, nq_))
        return carry

    def slow_attention():
        def head(h, carry):
            g = h // 8
            qm_s[...] = jnp.zeros(qm_s.shape, BF16)
            qm_s[pl.ds(pl.multiple_of((h % 8) * DH, DH), DH), :] = qt_s[pl.ds(pl.multiple_of(h * DH, DH), DH), pl.ds(q0, TQ)]

            def mx(c, m_acc):
                r0 = pl.multiple_of(c * TK, TK)
                s = _dot(k_s[g, pl.ds(r0, TK), :], qm_s[...])
                return jnp.maximum(m_acc, jnp.max(s, axis=0, keepdims=True))
            m = jax.lax.fori_loop(0, NC, mx, jnp.full((1, TQ), -jnp.inf, F32))

            def acc(c, lo):
                l_acc, o_acc = lo
                r0 = pl.multiple_of(c * TK, TK)
                s = _dot(k_s[g, pl.ds(r0, TK), :], qm_s[...])
                p = jnp.exp2(s - m)
                vt = vt_s[pl.ds(pl.multiple_of(h * DH, DH), DH), pl.ds(r0, TK)]
                return (l_acc + p.reshape(TK // 8, 8, TQ).sum(0), o_acc + _dot(vt, p.astype(BF16)))
            l_acc, o_acc = jax.lax.fori_loop(0, NC, acc, (jnp.zeros((8, TQ), F32), jnp.zeros((DH, TQ), F32)))
            finalize(h, l_acc, o_acc)
            lraw_s[...] = l_acc
            o_s[...] = o_acc
            return carry
        jax.lax.fori_loop(0, H, head, 0)
        for g in range(3):
            untranspose(g)

    def attempt(state):
        a, _ = state

        @pl.when(a == 0)
        def _():
            jax.lax.fori_loop(0, NG, fast_body, 0)

        @pl.when(a == 1)
        def _():
            slow_attention()

        @pl.when(jnp.logical_or(step > 0, a > 0))
        def _():
            prev = jnp.where(a > 0, step, jnp.maximum(step - 1, 0))
            for r in range(NO):
                out_copy(r, prev).wait()

        finalize(H - 1, lraw_s[...], o_s[...])
        untranspose(3)
        l_all = l_s[...]
        ok = jnp.logical_and(l_all >= L_LO, l_all <= L_HI)
        n_bad = jnp.sum(jnp.where(ok, 0.0, 1.0))
        o_fin = jnp.abs(ot_s[...].astype(F32)) <= 3.0e38
        n_bad = n_bad + jnp.sum(jnp.where(o_fin, 0.0, 1.0))

        nf = TQ // FC
        h1 = {}
        ln2 = {}
        act = {}
        for r in range(nf):
            rows = slice(r * FC, (r + 1) * FC)
            attn = None
            for g in range(4):
                part = _dot(on_s[g, rows, :], wo_v[128 * g:128 * (g + 1), :])
                attn = part if attn is None else attn + part
            h1[r] = x_v[pl.ds(pl.multiple_of(q0 + r * FC, FC), FC), :].astype(F32) + attn
            ln2[r] = _ln(h1[r]).astype(BF16)
        for r in range(nf):
            gate = _dot_nt(ln2[r], w1_v[...])
            up = _dot_nt(ln2[r], w3_v[...])
            act[r] = (gate * jax.nn.sigmoid(gate) * up).astype(BF16)
        for r in range(nf):
            for u in range(FC // OC):
                y = _dot(act[r][u * OC:(u + 1) * OC], w2_v[...])
                k = r * (FC // OC) + u
                out_v[k * OC:(k + 1) * OC, :] = (h1[r][u * OC:(u + 1) * OC] + y).astype(BF16)
                out_copy(k, step).start()
        redo = jnp.logical_or(n_bad > 0.0, flag_s[0] > 0)
        return a + 1, jnp.where(a == 0, redo.astype(jnp.int32), 0)

    jax.lax.while_loop(lambda s: s[0] < 1 + s[1], attempt, (jnp.int32(0), jnp.int32(0)))

    @pl.when(step == NQ - 1)
    def _():
        for r in range(NO):
            out_copy(r, step).wait()


@jax.jit
def pallas_sequential_preLN__softmax_full_mha__glu_gated_swiglu__prompt_kernel(
        A_x, A_wqkv, A_wo, B_x, B_w1, B_w3, B_w2):
    hbm = pl.BlockSpec(memory_space=pltpu.HBM)
    return pl.pallas_call(
        _kernel,
        grid=(NQ,),
        in_specs=[hbm] * 6,
        out_specs=hbm,
        out_shape=jax.ShapeDtypeStruct((1, S, D), BF16),
        scratch_shapes=[
            pltpu.VMEM((S, D), BF16),
            pltpu.VMEM((D, D), BF16),
            pltpu.VMEM((D, D), BF16),
            pltpu.VMEM((D, D), BF16),
            pltpu.VMEM((D, D), BF16),
            pltpu.VMEM((F, D), BF16),
            pltpu.VMEM((F, D), BF16),
            pltpu.VMEM((F, D), BF16),
            pltpu.VMEM((S, D), BF16),
            pltpu.VMEM((4, S, 128), BF16),
            pltpu.VMEM((S, D), F32),
            pltpu.VMEM((H // 2, S // 4, 128), U32),
            pltpu.VMEM((D, S), BF16),
            pltpu.VMEM((D, S), BF16),
            pltpu.VMEM((H, 32, S), U32),
            pltpu.VMEM((H, 8, S), F32),
            pltpu.VMEM((128, TQ), BF16),
            pltpu.VMEM((D, TQ), BF16),
            pltpu.VMEM((4, TQ, 128), BF16),
            pltpu.VMEM((H, TQ), F32),
            pltpu.VMEM((DH, TQ), F32),
            pltpu.VMEM((8, TQ), F32),
            pltpu.VMEM((DEPTH - 1, TK, TQ), I32),
            pltpu.VMEM((TK, TQ), BF16),
            pltpu.VMEM((8, TQ), F32),
            pltpu.VMEM((8, D), F32),
            pltpu.VMEM((D, 128), F32),
            pltpu.VMEM((TQ, D), BF16),
            pltpu.SMEM((HPB * NC,), jnp.int32),
            pltpu.SMEM((1,), jnp.int32),
            pltpu.SemaphoreType.DMA((NX + 7,)),
            pltpu.SemaphoreType.DMA((NO,)),
        ],
        compiler_params=pltpu.CompilerParams(
            dimension_semantics=("arbitrary",), vmem_limit_bytes=100 * 1024 * 1024),
        name="fused_block",
    )(A_x, A_wqkv, A_wo, B_w1.T, B_w3.T, B_w2)
```
